```python
import jax
import jax.numpy as jnp

def _softmax(x, axis=-1):
    return jax.nn.softmax(x, axis=axis)

def _gelu(x):
    return jax.nn.gelu(x, approximate=True)

def _silu(x):
    return jax.nn.silu(x)

def _sigmoid(x):
    return jax.nn.sigmoid(x)

def _layernorm(x, axis=-1, eps=1e-05):
    m = jnp.mean(x, axis=axis, keepdims=True)
    v = jnp.var(x, axis=axis, keepdims=True)
    return (x - m) / jnp.sqrt(v + eps)

def _scatter_add(tgt, idx, src, axis=0):
    return tgt.at[idx].add(src)

def _segment_sum(src, seg, n):
    return jax.ops.segment_sum(src, seg, n)

class _Rng:

    def __init__(self, key):
        self._k = key

    def _next(self):
        self._k, sub = jax.random.split(self._k)
        return sub

    def normal(self, shape):
        return jax.random.normal(self._next(), shape, dtype=jnp.bfloat16)

    def randint(self, lo, hi, shape):
        return jax.random.randint(self._next(), shape, lo, hi, dtype=jnp.int32)

    def uniform(self, shape, lo=0.0, hi=1.0):
        return jax.random.uniform(self._next(), shape, jnp.bfloat16, lo, hi)

    def permutation(self, n):
        return jax.random.permutation(self._next(), n)
kernel_name = 'parallel_sum__memory_aug_infini_attn__moe_arch_mod__prompt'

def setup_inputs():
    _rng = _Rng(jax.random.key(int.from_bytes(__import__("os").urandom(4), "little")))
    _w = lambda a: (lambda t: t.astype(jnp.bfloat16) if jnp.issubdtype(t.dtype, jnp.floating) else t)(jnp.asarray(a))

    def _A_setup():
        B, S, D, H = (1, 2048, 576, 32)
        N = 4
        L = max(1, S // N)
        sc = D ** (-0.5)
        return {'x': _w((lambda *s: _rng.normal(s) * 0.05)(B, N * L, D)), 'wq': _w((lambda *s: _rng.normal(s) * 0.05)(D, D) * sc), 'wk': _w((lambda *s: _rng.normal(s) * 0.05)(D, D) * sc), 'wv': _w((lambda *s: _rng.normal(s) * 0.05)(D, D) * sc), 'wo': _w((lambda *s: _rng.normal(s) * 0.05)(D, D) * sc), 'beta': _w((lambda *s: _rng.normal(s) * 0.05)(H))}
    _A_in = _A_setup()

    def _B_setup():
        B, S, D, F, C = (1, 2048, 576, 4608, 2)
        return {'x': _w((lambda *s: _rng.normal(s) * 0.05)(B, S, D)), 'w_r': _w((lambda *s: _rng.normal(s) * 0.05)(D)), 'w_gate': _w((lambda *s: _rng.normal(s) * 0.05)(D, F)), 'w_up': _w((lambda *s: _rng.normal(s) * 0.05)(D, F)), 'w_down': _w((lambda *s: _rng.normal(s) * 0.05)(F, D))}
    _B_in = _B_setup()
    return {'A_x': _A_in['x'], 'A_wq': _A_in['wq'], 'A_wk': _A_in['wk'], 'A_wv': _A_in['wv'], 'A_wo': _A_in['wo'], 'A_beta': _A_in['beta'], 'B_x': _B_in['x'], 'B_w_r': _B_in['w_r'], 'B_w_gate': _B_in['w_gate'], 'B_w_up': _B_in['w_up'], 'B_w_down': _B_in['w_down']}

def reference(A_x, A_wq, A_wk, A_wv, A_wo, A_beta, B_x, B_w_r, B_w_gate, B_w_up, B_w_down):

    def _A_ref(x, wq, wk, wv, wo, beta):
        B, S, D = x.shape
        H = 32
        Dh = D // H
        N = 4
        L = S // N
        q = (lambda x, *d: x.transpose(*d))((x @ wq).reshape(B, S, H, Dh), 0, 2, 1, 3).reshape(B, H, N, L, Dh)
        k = (lambda x, *d: x.transpose(*d))((x @ wk).reshape(B, S, H, Dh), 0, 2, 1, 3).reshape(B, H, N, L, Dh)
        v = (lambda x, *d: x.transpose(*d))((x @ wv).reshape(B, S, H, Dh), 0, 2, 1, 3).reshape(B, H, N, L, Dh)
        phi = lambda t: jnp.where(t > 0, t + 1.0, jnp.exp(t))
        scale = Dh ** (-0.5)
        ar = jnp.arange(L)
        mask = (lambda x, dt: x.astype(dt))(ar[:, None] < ar[None, :], x.dtype) * -1000000000.0
        g = _sigmoid(beta).reshape(1, H, 1, 1)
        M = jnp.einsum('bhd,bhe->bhde', q[:, :, 0, 0, :] * 0.0, q[:, :, 0, 0, :] * 0.0)
        z = q[:, :, 0, 0, :] * 0.0
        outs = []
        for s in range(N):
            qs, ks, vs = (q[:, :, s].copy(), k[:, :, s].copy(), v[:, :, s].copy())
            logits = jnp.einsum('bhqd,bhkd->bhqk', qs, ks) * scale + mask
            p = _softmax(logits, axis=-1)
            a_dot = jnp.einsum('bhqk,bhkd->bhqd', p, vs)
            pq = phi(qs)
            num = jnp.einsum('bhld,bhde->bhle', pq, M)
            den = jnp.einsum('bhld,bhd->bhl', pq, z)[..., None] + 1e-06
            a_mem = num / den
            o = g * a_mem + (1.0 - g) * a_dot
            outs.append(o)
            pk = phi(ks)
            M = M + jnp.einsum('bhld,bhle->bhde', pk, vs)
            z = z + jnp.einsum('bhld->bhd', pk)
        o = (lambda x, *d: x.transpose(*d))(jnp.stack(outs, 2).reshape(B, H, S, Dh), 0, 2, 1, 3).reshape(B, S, D)
        return o @ wo

    def _B_ref(x, w_r, w_gate, w_up, w_down):
        B, S, D = x.shape
        C = 2
        r = x @ w_r
        idx = jnp.argsort(-r, axis=-1)[:, :C]
        idx_e = jnp.repeat(idx.reshape(B, C, 1), D, axis=2)
        x_sel = jnp.take_along_axis(x, idx_e, axis=1)
        g = _silu(x_sel @ w_gate)
        u = x_sel @ w_up
        y = g * u @ w_down
        r_sel = _sigmoid(jnp.take_along_axis(r, idx, axis=1))
        y = y * r_sel.reshape(B, C, 1)
        b_off = (jnp.arange(B) * S).reshape(B, 1)
        flat_idx = (idx + b_off).reshape(B * C)
        zero = (x * 0.0).reshape(B * S, D)
        upd = _scatter_add(zero, flat_idx, y.reshape(B * C, D), axis=0)
        return x + upd.reshape(B, S, D)
    x = A_x
    xn = _layernorm(x, axis=-1)
    return x + _A_ref(xn, A_wq, A_wk, A_wv, A_wo, A_beta) + _B_ref(xn, B_w_r, B_w_gate, B_w_up, B_w_down)
```

```python
import functools
import math

import jax
import jax.numpy as jnp
import jax.experimental.pallas as pl
import jax.experimental.pallas.tpu as pltpu

D = 576
S = 2048
H = 32
DH = D // H
NSEG = 4
L = S // NSEG
FF = 4608
HG = 4
NG = H // HG
GR = HG * DH
GP = 80
T = 128
NT = L // T
CH = 2 * GR
DP = 640

F32 = jnp.float32
BF16 = jnp.bfloat16
QSCALE = (DH ** -0.5) * math.log2(math.e)
NEG = -1e30


def _iota(shape, dim):
    return jax.lax.broadcasted_iota(jnp.int32, shape, dim)


def _round_bf16(t):
    return t.astype(BF16).astype(F32)


def _phi(t):
    return jnp.where(t > 0, t + 1.0, jnp.exp(t))


def _dot(a, b):
    return jnp.dot(a, b, preferred_element_type=F32)


def _dot_nt(a, b):
    return jax.lax.dot_general(a, b, (((1,), (1,)), ((), ())), preferred_element_type=F32)


def _kernel(wr_ref, beta_ref, x_hbm, wq_hbm, wk_hbm, wv_hbm, wo_hbm, wg_hbm, wu_hbm, wd_hbm,
            out_hbm,
            x_v, wraw_v, wo_v, wt_v, wot_v, xn_v, qs_v, pq_v, kn_v, vt_v, ot_v, r_v, gate_v,
            wg_v, wu_v, wd_v, out_v, in_sem, out_sem):
    x_cp = [pltpu.make_async_copy(x_hbm.at[:, pl.ds(s * L, L)], x_v.at[s], in_sem.at[s])
            for s in range(NSEG)]
    w_cp = [pltpu.make_async_copy(w, wraw_v.at[i], in_sem.at[NSEG + i])
            for i, w in enumerate((wq_hbm, wk_hbm, wv_hbm))]
    wo_cp = pltpu.make_async_copy(wo_hbm, wo_v.at[pl.ds(0, D)], in_sem.at[NSEG + 3])
    f_cp = [pltpu.make_async_copy(src, dst, in_sem.at[NSEG + 4 + i])
            for i, (src, dst) in enumerate(((wg_hbm, wg_v), (wu_hbm, wu_v), (wd_hbm, wd_v)))]
    x_cp[0].start()
    for c in w_cp:
        c.start()
    for c in x_cp[1:]:
        c.start()

    sg = jax.nn.sigmoid(beta_ref[...].astype(F32).reshape(1, H))
    diag = jnp.where(_iota((H, H), 0) == _iota((H, H), 1), jnp.broadcast_to(sg, (H, H)), 0.0)
    gate_v[...] = jnp.broadcast_to(jnp.sum(diag, axis=1, keepdims=True), (H, T))
    wt_v[pl.ds(3 * D, 16), :] = jnp.broadcast_to(
        wr_ref[...].astype(F32).reshape(1, D), (16, D)).astype(BF16)

    def layernorm(s):
        for t in range(NT):
            x = x_v[s, :, pl.ds(t * T, T)].astype(F32)
            m = jnp.sum(x, axis=0, keepdims=True) * (1.0 / D)
            xc = x - m
            v = jnp.sum(xc * xc, axis=0, keepdims=True) * (1.0 / D)
            sd = _round_bf16(jnp.sqrt(_round_bf16(_round_bf16(v) + 1e-5)))
            xn_v[s, :, pl.ds(t * T, T)] = (_round_bf16(x - _round_bf16(m)) * (1.0 / sd)).astype(BF16)

    x_cp[0].wait()
    layernorm(0)
    for i in range(3):
        w_cp[i].wait()
        wt_v[pl.ds(i * D, D), :] = wraw_v[i].T
    for s in range(1, NSEG):
        x_cp[s].wait()
    wo_cp.start()
    for c in f_cp:
        c.start()
    for s in range(1, NSEG):
        layernorm(s)

    def project(s, carry):
        xn = xn_v[s]
        zpad = jnp.zeros((GP - GR, L), F32)
        for p in range(NG // 2):
            q = _dot(wt_v[pl.ds(p * CH, CH), :], xn)
            pq = _phi(q)
            q = q * QSCALE
            for j in range(2):
                rows = slice(j * GR, (j + 1) * GR)
                qs_v[s, 2 * p + j] = jnp.concatenate([q[rows], zpad], axis=0).astype(BF16)
                pq_v[s, 2 * p + j] = jnp.concatenate([pq[rows], zpad], axis=0).astype(BF16)
            k = _dot(wt_v[pl.ds(D + p * CH, CH), :], xn)
            for j in range(2):
                kg = jnp.concatenate([k[j * GR:(j + 1) * GR], jnp.zeros((T - GR, L), F32)], axis=0)
                kn_v[s, 2 * p + j] = kg.astype(BF16).T
            extra = 16 if p == NG // 2 - 1 else 0
            v = _dot(wt_v[pl.ds(2 * D + p * CH, CH + extra), :], xn)
            for j in range(2):
                vt_v[s, 2 * p + j, pl.ds(0, GR), :] = v[j * GR:(j + 1) * GR]
                vt_v[s, 2 * p + j, pl.ds(GR, GP - GR), :] = jnp.ones((GP - GR, L), F32)
            if extra:
                r_v[s] = v[CH:CH + 8]
        return carry

    jax.lax.fori_loop(0, NSEG, project, 0)

    def attend(g, carry):
        row = _iota((GP, T), 0)
        lane = _iota((GP, T), 1)
        mz_mask = jnp.zeros((GP, T), jnp.bool_)
        for h in range(HG):
            in_row = ((row >= h * DH) & (row < (h + 1) * DH)) | (row == GR + h)
            mz_mask = mz_mask | (in_row & (lane >= h * DH) & (lane < (h + 1) * DH))
        causal = _iota((T, T), 0) <= _iota((T, T), 1)
        row8 = _iota((8, T), 0)
        row8l = _iota((8, L), 0)
        gates = [gate_v[pl.ds(g * HG + h, 1), :] for h in range(HG)]
        mz = None
        for s in range(NSEG):
            if s > 0:
                mem = _dot(mz[:, :GP].astype(BF16), pq_v[s, g])
            vh = []
            for h in range(HG):
                w = vt_v[s, g, pl.ds(16 * h, 24), :]
                if h < HG - 1:
                    w = jnp.concatenate([w[:16], jnp.where(row8l == 7, 1.0, w[16:])], axis=0)
                else:
                    w = jnp.concatenate([jnp.where(row8l == 0, 1.0, w[:8]), w[8:]], axis=0)
                vh.append(w)
            for i in range(NT):
                qt = qs_v[s, g, :, pl.ds(i * T, T)]
                outs = []
                for h in range(HG):
                    qm = jnp.where((row >= h * DH) & (row < (h + 1) * DH), qt, jnp.zeros_like(qt))
                    st = _dot(kn_v[s, g, pl.ds(0, (i + 1) * T), pl.ds(0, GP)], qm)
                    blocks = [st[j * T:(j + 1) * T] for j in range(i + 1)]
                    blocks[i] = jnp.where(causal, blocks[i], NEG)
                    st = jnp.concatenate(blocks, axis=0) if i else blocks[0]
                    m = jnp.max(st, axis=0, keepdims=True)
                    acc = _dot(vh[h][:, :(i + 1) * T], jnp.exp2(st - m))
                    lrow = 23 if h < HG - 1 else 0
                    o = acc * ((1.0 - gates[h]) / acc[lrow:lrow + 1])
                    if s > 0:
                        mt = mem[:, i * T:(i + 1) * T]
                        o = o + mt[16 * h:16 * h + 24] * (gates[h] / (mt[GR + h:GR + h + 1] + 1e-6))
                    outs.append(o)
                pieces = [outs[0][:16]]
                for h in range(1, HG):
                    pieces.append(jnp.where(row8 < 2 * h, outs[h - 1][16:], outs[h][:8]))
                    pieces.append(outs[h][8:16] if h < HG - 1 else outs[h][8:])
                ot_v[s, pl.ds(pl.multiple_of(g * GR, 8), GR), pl.ds(i * T, T)] = (
                    jnp.concatenate(pieces, axis=0))
            if s < NSEG - 1:
                upd = jnp.where(mz_mask, _dot(vt_v[s, g], _phi(kn_v[s, g].astype(F32))), 0.0)
                mz = upd if mz is None else mz + upd
        return carry

    jax.lax.fori_loop(0, NG, attend, 0)

    r = _round_bf16(jnp.concatenate([r_v[s] for s in range(NSEG)], axis=1))
    pos = _iota((8, S), 1)
    m1 = jnp.max(r, axis=1, keepdims=True)
    i1 = jnp.min(jnp.where(r == m1, pos, S), axis=1, keepdims=True)
    r2 = jnp.where(pos == i1, -jnp.inf, r)
    m2 = jnp.max(r2, axis=1, keepdims=True)
    i2 = jnp.min(jnp.where((r2 == m2) & (pos != i1), pos, S), axis=1, keepdims=True)
    sub = _iota((8, S), 0)
    onehot = ((sub == 0) & (pos == i1)) | ((sub == 1) & (pos == i2))
    onehot = jnp.concatenate([jnp.where(onehot, 1.0, 0.0), jnp.zeros((8, S), F32)], axis=0)
    for s in range(NSEG):
        ot_v[s, pl.ds(D, 16), :] = onehot[:, s * L:(s + 1) * L]
        ot_v[s, pl.ds(D + 16, DP - D - 16), :] = jnp.zeros((DP - D - 16, L), F32)
    xsel = _dot_nt(onehot[:, :L].astype(BF16), xn_v[0])
    for s in range(1, NSEG):
        xsel = xsel + _dot_nt(onehot[:, s * L:(s + 1) * L].astype(BF16), xn_v[s])
    xsel = xsel.astype(BF16)
    for c in f_cp:
        c.wait()
    a = _dot(xsel, wg_v[...])
    u = _dot(xsel, wu_v[...])
    hid = (a * jax.nn.sigmoid(a) * u).astype(BF16)
    y = _dot_nt(hid, wd_v[...])
    rsel = jax.nn.sigmoid(jnp.where(_iota((8, 1), 0) == 0, m1, m2))
    y = jnp.concatenate([y[:8] * rsel, jnp.zeros((8, D), F32)], axis=0)

    wo_cp.wait()
    wo_v[pl.ds(D, 16), :] = y.astype(BF16)
    wo_v[pl.ds(D + 16, DP - D - 16), :] = jnp.zeros((DP - D - 16, D), BF16)
    wot_v[...] = wo_v[...].T

    def out_copy(s):
        return pltpu.make_async_copy(out_v.at[s], out_hbm.at[:, pl.ds(s * L, L)], out_sem.at[s])

    for s in range(NSEG):
        att = _dot(wot_v[...], ot_v[s].astype(BF16))
        out_v[s] = (x_v[s].astype(F32) + att + xn_v[s].astype(F32)).astype(BF16)
        out_copy(s).start()
    for s in range(NSEG):
        out_copy(s).wait()


@jax.jit
def pallas_parallel_sum__memory_aug_infini_attn__moe_arch_mod__prompt_kernel(
    A_x: jax.Array,
    A_wq: jax.Array,
    A_wk: jax.Array,
    A_wv: jax.Array,
    A_wo: jax.Array,
    A_beta: jax.Array,
    B_x: jax.Array,
    B_w_r: jax.Array,
    B_w_gate: jax.Array,
    B_w_up: jax.Array,
    B_w_down: jax.Array,
):
    del B_x
    assert A_x.shape == (1, S, D) and B_w_gate.shape == (D, FF)
    hbm = pl.BlockSpec(memory_space=pl.ANY)
    vmem = pl.BlockSpec(memory_space=pltpu.VMEM)
    out_t = pl.pallas_call(
        _kernel,
        out_shape=jax.ShapeDtypeStruct((D, S), BF16),
        in_specs=[vmem, vmem] + [hbm] * 8,
        out_specs=hbm,
        scratch_shapes=[
            pltpu.VMEM((NSEG, D, L), BF16),
            pltpu.VMEM((3, D, D), BF16),
            pltpu.VMEM((DP, D), BF16),
            pltpu.VMEM((3 * D + 16, D), BF16),
            pltpu.VMEM((D, DP), BF16),
            pltpu.VMEM((NSEG, D, L), BF16),
            pltpu.VMEM((NSEG, NG, GP, L), BF16),
            pltpu.VMEM((NSEG, NG, GP, L), BF16),
            pltpu.VMEM((NSEG, NG, L, T), BF16),
            pltpu.VMEM((NSEG, NG, GP, L), F32),
            pltpu.VMEM((NSEG, DP, L), F32),
            pltpu.VMEM((NSEG, 8, L), F32),
            pltpu.VMEM((H, T), F32),
            pltpu.VMEM((D, FF), BF16),
            pltpu.VMEM((D, FF), BF16),
            pltpu.VMEM((D, FF), BF16),
            pltpu.VMEM((NSEG, D, L), BF16),
            pltpu.SemaphoreType.DMA((NSEG + 7,)),
            pltpu.SemaphoreType.DMA((NSEG,)),
        ],
        compiler_params=pltpu.CompilerParams(vmem_limit_bytes=100 * 2 ** 20),
        name="infini_mod",
    )(B_w_r, A_beta, A_x[0].T, A_wq, A_wk, A_wv, A_wo, B_w_gate, B_w_up, B_w_down.T)
    return out_t.T[None]
```

```python
import functools
import math

import jax
import jax.numpy as jnp
import jax.experimental.pallas as pl
import jax.experimental.pallas.tpu as pltpu

D = 576
S = 2048
H = 32
DH = D // H
NSEG = 4
L = S // NSEG
FF = 4608
HG = 4
NG = H // HG
GR = HG * DH
GP = 80
T = 128
NT = L // T
CH = 2 * GR
DP = 640

F32 = jnp.float32
BF16 = jnp.bfloat16
QSCALE = (DH ** -0.5) * math.log2(math.e)
NEG = -1e30
LAG = 5
RING = 8
SCR = True


def _iota(shape, dim):
    return jax.lax.broadcasted_iota(jnp.int32, shape, dim)


def _round_bf16(t):
    return t.astype(BF16).astype(F32)


def _phi(t):
    return jnp.where(t > 0, t + 1.0, jnp.exp(t))


def _dot(a, b):
    return jnp.dot(a, b, preferred_element_type=F32)


def _dot_nt(a, b):
    return jax.lax.dot_general(a, b, (((1,), (1,)), ((), ())), preferred_element_type=F32)


def _kernel(wr_ref, beta_ref, x_hbm, wq_hbm, wk_hbm, wv_hbm, wo_hbm, wg_hbm, wu_hbm, wd_hbm,
            out_hbm,
            x_v, wraw_v, wo_v, wt_v, wot_v, xn_v, qs_v, pq_v, kn_v, vt_v, ot_v, r_v, gate_v, bias_v, st_v,
            wg_v, wu_v, wd_v, out_v, in_sem, out_sem):
    x_cp = [pltpu.make_async_copy(x_hbm.at[:, pl.ds(s * L, L)], x_v.at[s], in_sem.at[s])
            for s in range(NSEG)]
    w_cp = [pltpu.make_async_copy(w, wraw_v.at[i], in_sem.at[NSEG + i])
            for i, w in enumerate((wq_hbm, wk_hbm, wv_hbm))]
    wo_cp = pltpu.make_async_copy(wo_hbm, wo_v.at[pl.ds(0, D)], in_sem.at[NSEG + 3])
    f_cp = [pltpu.make_async_copy(src, dst, in_sem.at[NSEG + 4 + i])
            for i, (src, dst) in enumerate(((wg_hbm, wg_v), (wu_hbm, wu_v), (wd_hbm, wd_v)))]
    x_cp[0].start()
    for c in w_cp:
        c.start()
    for c in x_cp[1:]:
        c.start()

    sg = jax.nn.sigmoid(beta_ref[...].astype(F32).reshape(1, H))
    diag = jnp.where(_iota((H, H), 0) == _iota((H, H), 1), jnp.broadcast_to(sg, (H, H)), 0.0)
    gate_v[...] = jnp.broadcast_to(jnp.sum(diag, axis=1, keepdims=True), (H, T))
    wt_v[pl.ds(3 * D, 16), :] = jnp.broadcast_to(
        wr_ref[...].astype(F32).reshape(1, D), (16, D)).astype(BF16)

    def layernorm(s):
        for t in range(NT):
            x = x_v[s, :, pl.ds(t * T, T)].astype(F32)
            m = jnp.sum(x, axis=0, keepdims=True) * (1.0 / D)
            xc = x - m
            v = jnp.sum(xc * xc, axis=0, keepdims=True) * (1.0 / D)
            sd = _round_bf16(jnp.sqrt(_round_bf16(_round_bf16(v) + 1e-5)))
            xn_v[s, :, pl.ds(t * T, T)] = (_round_bf16(x - _round_bf16(m)) * (1.0 / sd)).astype(BF16)

    x_cp[0].wait()
    layernorm(0)
    for i in range(3):
        w_cp[i].wait()
        wt_v[pl.ds(i * D, D), :] = wraw_v[i].T
    for s in range(1, NSEG):
        x_cp[s].wait()
    wo_cp.start()
    for c in f_cp:
        c.start()
    for s in range(1, NSEG):
        layernorm(s)

    def project(s, carry):
        xn = xn_v[s]
        zpad = jnp.zeros((GP - GR, L), F32)
        row32 = _iota((32, L), 0)
        for p in range(NG // 2):
            q = _dot(wt_v[pl.ds(p * CH, CH), :], xn)
            pq = _phi(q)
            q = q * QSCALE
            for j in range(2):
                rows = slice(j * GR, (j + 1) * GR)
                qg = jnp.concatenate([q[rows], zpad], axis=0)
                for h in range(HG):
                    keep = (row32 >= 2 * h) & (row32 < 2 * h + DH)
                    qs_v[s, 2 * p + j, h] = jnp.where(keep, qg[16 * h:16 * h + 32], 0.0).astype(BF16)
                pq_v[s, 2 * p + j] = jnp.concatenate([pq[rows], zpad], axis=0).astype(BF16)
            k = _dot(wt_v[pl.ds(D + p * CH, CH), :], xn)
            for j in range(2):
                kg = jnp.concatenate([k[j * GR:(j + 1) * GR], jnp.zeros((T - GR, L), F32)], axis=0)
                kn_v[s, 2 * p + j] = kg.astype(BF16).T
            extra = 16 if p == NG // 2 - 1 else 0
            v = _dot(wt_v[pl.ds(2 * D + p * CH, CH + extra), :], xn)
            for j in range(2):
                vt_v[s, 2 * p + j, pl.ds(0, GR), :] = v[j * GR:(j + 1) * GR]
                vt_v[s, 2 * p + j, pl.ds(GR, GP - GR), :] = jnp.ones((GP - GR, L), F32)
            if extra:
                r_v[s] = v[CH:CH + 8]
        return carry

    jax.lax.fori_loop(0, NSEG, project, 0)

    bias_v[...] = jnp.where(_iota((T, T), 0) <= _iota((T, T), 1), 0.0, NEG)
    blocks = [(s, i, j) for s in range(NSEG) for i in reversed(range(NT)) for j in range(i + 1)]

    def attend(g, carry):
        row = _iota((GP, T), 0)
        lane = _iota((GP, T), 1)
        mz_mask = jnp.zeros((GP, T), jnp.bool_)
        for h in range(HG):
            in_row = ((row >= h * DH) & (row < (h + 1) * DH)) | (row == GR + h)
            mz_mask = mz_mask | (in_row & (lane >= h * DH) & (lane < (h + 1) * DH))
        row8 = _iota((8, T), 0)
        gates = [gate_v[pl.ds(g * HG + h, 1), :] for h in range(HG)]
        lrow = [23, 23, 23, 0]
        st, run_max, col_max, acc, mem, mz = {}, {}, {}, {}, {}, [None]

        def scores(n):
            s, i, j = blocks[n]
            kt = kn_v[s, g, pl.ds(j * T, T), :]
            for h in range(HG):
                parts = [qs_v[s, g, h, :, pl.ds(i * T, T)], jnp.zeros((T - 32 - 16 * h, T), BF16)]
                if h:
                    parts.insert(0, jnp.zeros((16 * h, T), BF16))
                t = _dot(kt, jnp.concatenate(parts, axis=0))
                if j == i:
                    t = t + bias_v[...]
                if SCR:
                    st_v[n % RING, h] = t
                else:
                    st[n, h] = t
                m = jnp.max(t.reshape(T // 8, 8, T), axis=0)
                run_max[h] = m if j == 0 else jnp.maximum(run_max[h], m)
                if j == i:
                    col_max[s, i, h] = jnp.max(run_max[h], axis=0, keepdims=True)

        def values(n):
            s, i, j = blocks[n]
            for h in range(HG):
                w = vt_v[s, g, pl.ds(16 * h, 24), pl.ds(j * T, T)]
                if h < HG - 1:
                    w = jnp.concatenate([w[:16], jnp.where(row8 == 7, 1.0, w[16:])], axis=0)
                else:
                    w = jnp.concatenate([jnp.where(row8 == 0, 1.0, w[:8]), w[8:]], axis=0)
                t = st_v[n % RING, h] if SCR else st.pop((n, h))
                a = _dot(w, jnp.exp2(t - col_max[s, i, h]))
                acc[h] = a if j == 0 else acc[h] + a
            if j < i:
                return
            if s > 0:
                mt = _dot(mz[0][s - 1], pq_v[s, g, :, pl.ds(i * T, T)])
            outs = []
            for h in range(HG):
                o = acc[h] * ((1.0 - gates[h]) / acc[h][lrow[h]:lrow[h] + 1])
                if s > 0:
                    o = o + mt[16 * h:16 * h + 24] * (gates[h] / (mt[GR + h:GR + h + 1] + 1e-6))
                outs.append(o)
            pieces = [outs[0][:16]]
            for h in range(1, HG):
                pieces.append(jnp.where(row8 < 2 * h, outs[h - 1][16:], outs[h][:8]))
                pieces.append(outs[h][8:16] if h < HG - 1 else outs[h][8:])
            ot_v[s, pl.ds(pl.multiple_of(g * GR, 8), GR), pl.ds(i * T, T)] = (
                jnp.concatenate(pieces, axis=0))

        def memories():
            out, run = [], None
            for s in range(NSEG - 1):
                upd = jnp.where(mz_mask, _dot(vt_v[s, g], _phi(kn_v[s, g].astype(F32))), 0.0)
                run = upd if run is None else run + upd
                out.append(run[:, :GP].astype(BF16))
            mz[0] = out

        memories()
        for n in range(len(blocks) + LAG):
            if n < len(blocks):
                scores(n)
            if n >= LAG:
                values(n - LAG)
        return carry

    jax.lax.fori_loop(0, NG, attend, 0)

    r = _round_bf16(jnp.concatenate([r_v[s] for s in range(NSEG)], axis=1))
    pos = _iota((8, S), 1)
    m1 = jnp.max(r, axis=1, keepdims=True)
    i1 = jnp.min(jnp.where(r == m1, pos, S), axis=1, keepdims=True)
    r2 = jnp.where(pos == i1, -jnp.inf, r)
    m2 = jnp.max(r2, axis=1, keepdims=True)
    i2 = jnp.min(jnp.where((r2 == m2) & (pos != i1), pos, S), axis=1, keepdims=True)
    sub = _iota((8, S), 0)
    onehot = ((sub == 0) & (pos == i1)) | ((sub == 1) & (pos == i2))
    onehot = jnp.concatenate([jnp.where(onehot, 1.0, 0.0), jnp.zeros((8, S), F32)], axis=0)
    for s in range(NSEG):
        ot_v[s, pl.ds(D, 16), :] = onehot[:, s * L:(s + 1) * L]
        ot_v[s, pl.ds(D + 16, DP - D - 16), :] = jnp.zeros((DP - D - 16, L), F32)
    xsel = _dot_nt(onehot[:, :L].astype(BF16), xn_v[0])
    for s in range(1, NSEG):
        xsel = xsel + _dot_nt(onehot[:, s * L:(s + 1) * L].astype(BF16), xn_v[s])
    xsel = xsel.astype(BF16)
    for c in f_cp:
        c.wait()
    a = _dot(xsel, wg_v[...])
    u = _dot(xsel, wu_v[...])
    hid = (a * jax.nn.sigmoid(a) * u).astype(BF16)
    y = _dot_nt(hid, wd_v[...])
    rsel = jax.nn.sigmoid(jnp.where(_iota((8, 1), 0) == 0, m1, m2))
    y = jnp.concatenate([y[:8] * rsel, jnp.zeros((8, D), F32)], axis=0)

    wo_cp.wait()
    wo_v[pl.ds(D, 16), :] = y.astype(BF16)
    wo_v[pl.ds(D + 16, DP - D - 16), :] = jnp.zeros((DP - D - 16, D), BF16)
    wot_v[...] = wo_v[...].T

    def out_copy(s):
        return pltpu.make_async_copy(out_v.at[s], out_hbm.at[:, pl.ds(s * L, L)], out_sem.at[s])

    for s in range(NSEG):
        att = _dot(wot_v[...], ot_v[s].astype(BF16))
        out_v[s] = (x_v[s].astype(F32) + att + xn_v[s].astype(F32)).astype(BF16)
        out_copy(s).start()
    for s in range(NSEG):
        out_copy(s).wait()


@jax.jit
def pallas_parallel_sum__memory_aug_infini_attn__moe_arch_mod__prompt_kernel(
    A_x: jax.Array,
    A_wq: jax.Array,
    A_wk: jax.Array,
    A_wv: jax.Array,
    A_wo: jax.Array,
    A_beta: jax.Array,
    B_x: jax.Array,
    B_w_r: jax.Array,
    B_w_gate: jax.Array,
    B_w_up: jax.Array,
    B_w_down: jax.Array,
):
    del B_x
    assert A_x.shape == (1, S, D) and B_w_gate.shape == (D, FF)
    hbm = pl.BlockSpec(memory_space=pl.ANY)
    vmem = pl.BlockSpec(memory_space=pltpu.VMEM)
    out_t = pl.pallas_call(
        _kernel,
        out_shape=jax.ShapeDtypeStruct((D, S), BF16),
        in_specs=[vmem, vmem] + [hbm] * 8,
        out_specs=hbm,
        scratch_shapes=[
            pltpu.VMEM((NSEG, D, L), BF16),
            pltpu.VMEM((3, D, D), BF16),
            pltpu.VMEM((DP, D), BF16),
            pltpu.VMEM((3 * D + 16, D), BF16),
            pltpu.VMEM((D, DP), BF16),
            pltpu.VMEM((NSEG, D, L), BF16),
            pltpu.VMEM((NSEG, NG, HG, 32, L), BF16),
            pltpu.VMEM((NSEG, NG, GP, L), BF16),
            pltpu.VMEM((NSEG, NG, L, T), BF16),
            pltpu.VMEM((NSEG, NG, GP, L), F32),
            pltpu.VMEM((NSEG, DP, L), F32),
            pltpu.VMEM((NSEG, 8, L), F32),
            pltpu.VMEM((H, T), F32),
            pltpu.VMEM((T, T), F32),
            pltpu.VMEM((RING, HG, T, T), F32),
            pltpu.VMEM((D, FF), BF16),
            pltpu.VMEM((D, FF), BF16),
            pltpu.VMEM((D, FF), BF16),
            pltpu.VMEM((NSEG, D, L), BF16),
            pltpu.SemaphoreType.DMA((NSEG + 7,)),
            pltpu.SemaphoreType.DMA((NSEG,)),
        ],
        compiler_params=pltpu.CompilerParams(vmem_limit_bytes=100 * 2 ** 20),
        name="infini_mod",
    )(B_w_r, A_beta, A_x[0].T, A_wq, A_wk, A_wv, A_wo, B_w_gate, B_w_up, B_w_down.T)
    return out_t.T[None]
```

```python
import math
from functools import partial

import jax
import jax.numpy as jnp
import jax.experimental.pallas as pl
import jax.experimental.pallas.tpu as pltpu

D = 576
S = 2048
H = 32
DH = D // H
NSEG = 4
L = S // NSEG
FF = 4608
HG = 4
NG = H // HG
GR = HG * DH
GP = 80
T = 128
NT = L // T
CH = 2 * GR
DP = 640
FT = FF // T // (NG - 2)

F32 = jnp.float32
BF16 = jnp.bfloat16
U32 = jnp.uint32
QSCALE = (DH ** -0.5) * math.log2(math.e)
NEG = -1e30
SAFE_LO, SAFE_HI = 2.0 ** -30, 2.0 ** 30
LAG = 2
UNR = 1
FCH = 2


def _iota(shape, dim):
    return jax.lax.broadcasted_iota(jnp.int32, shape, dim)


def _round_bf16(t):
    return t.astype(BF16).astype(F32)


def _pack(t):
    return pltpu.bitcast(t.astype(BF16), U32)


def _bf(t):
    return pltpu.bitcast(t, BF16)


def _phi(t):
    return jnp.where(t > 0, t + 1.0, jnp.exp(t))


def _dot(a, b):
    return jax.lax.dot_general(a, b, (((1,), (0,)), ((), ())), preferred_element_type=F32)


def _aligned(i, n):
    return i if isinstance(i, int) else pl.multiple_of(i, n)


def _kernel(wr_hbm, beta_hbm, x_hbm, wq_hbm, wk_hbm, wv_hbm, wo_hbm, wg_hbm, wu_hbm, wd_hbm,
            out_hbm,
            wr_v, beta_v, x_v, wraw_v, wo_v, wt_v, wot_v, xn_v, qs_v, pq_v, kn_v, vt_v, ot_v,
            r_v, gate_v, bias_v, lim_v, xs_v, y_v, rs_v, wg_v, wu_v, wd_v, out_v, in_sem, out_sem):
    x_cp = [pltpu.make_async_copy(x_hbm.at[:, pl.ds(s * L, L)], x_v.at[s], in_sem.at[s])
            for s in range(NSEG)]
    w_cp = [pltpu.make_async_copy(w, wraw_v.at[i], in_sem.at[NSEG + i])
            for i, w in enumerate((wq_hbm, wk_hbm, wv_hbm))]
    late_cp = [pltpu.make_async_copy(src, dst, in_sem.at[NSEG + 3 + i]) for i, (src, dst) in enumerate(
        ((wo_hbm, wo_v.at[pl.ds(0, D)]), (wg_hbm, wg_v), (wu_hbm, wu_v), (wd_hbm, wd_v)))]
    small_cp = [pltpu.make_async_copy(wr_hbm, wr_v, in_sem.at[NSEG + 7]),
                pltpu.make_async_copy(beta_hbm, beta_v, in_sem.at[NSEG + 8])]

    def layernorm(s, t):
        x = x_v[s, :, pl.ds(t * T, T)].astype(F32)
        xc = x - jnp.sum(x, axis=0, keepdims=True) * (1.0 / D)
        v = jnp.sum(xc * xc, axis=0, keepdims=True) * (1.0 / D)
        sd = _round_bf16(jnp.sqrt(_round_bf16(_round_bf16(v) + 1e-5)))
        xn_v[s, :, pl.ds(t * T, T)] = _pack(xc * (1.0 / sd))

    def transpose_weight(i, t):
        n = min(T, D - t * T)
        wt_v[pl.ds((i * D + t * T) // 2, n // 2), :] = pltpu.bitcast(
            wraw_v[i, :, pl.ds(t * T, n)].T, U32)

    def proj(s, row, n):
        return _dot(_bf(wt_v[pl.ds(row // 2, n // 2), :]), _bf(xn_v[s]))

    def project_q(s, p):
        zpad = jnp.zeros((GP - GR, L), F32)
        row32 = _iota((32, L), 0)
        q = proj(s, p * CH, CH)
        pq = _phi(q) if s else None
        q = q * QSCALE
        for j in range(2):
            rows = slice(j * GR, (j + 1) * GR)
            qg = jnp.concatenate([q[rows], zpad], axis=0)
            for h in range(HG):
                keep = (row32 >= 2 * h) & (row32 < 2 * h + DH)
                qs_v[s, 2 * p + j, h] = _pack(jnp.where(keep, qg[16 * h:16 * h + 32], 0.0))
            if s:
                pq_v[s, 2 * p + j] = _pack(jnp.concatenate([pq[rows], zpad], axis=0))

    def project_k(s, p):
        k = proj(s, D + p * CH, CH)
        for j in range(2):
            kg = jnp.concatenate([k[j * GR:(j + 1) * GR], jnp.zeros((T - GR, L), F32)], axis=0)
            kn_v[s, 2 * p + j] = pltpu.bitcast(kg.astype(BF16).T, U32)

    def project_v(s, p):
        extra = 16 if p == NG // 2 - 1 else 0
        v = proj(s, 2 * D + p * CH, CH + extra)
        for j in range(2):
            vt_v[s, 2 * p + j] = v[j * GR:(j + 1) * GR]
        if extra:
            r_v[s] = v[CH:CH + 8]

    def small_tables():
        wt_v[pl.ds(3 * D // 2, 8), :] = _pack(
            jnp.broadcast_to(wr_v[...].astype(F32).reshape(1, D), (16, D)))
        sg = jax.nn.sigmoid(beta_v[...].astype(F32).reshape(1, H))
        trow = _iota((NG * 8, H), 0)
        head = (trow >> 3) * HG + ((trow + jnp.where((trow & 4) != 0, 3, 0)) & 3)
        gcol = jnp.sum(jnp.where(_iota((NG * 8, H), 1) == head,
                                 jnp.broadcast_to(sg, (NG * 8, H)), 0.0), axis=1, keepdims=True)
        gcol = jnp.where((_iota((NG * 8, 1), 0) & 4) != 0, 1.0 - gcol, gcol)
        gate_v[...] = jnp.broadcast_to(gcol, (NG * 8, T))

    for c in [x_cp[0], w_cp[0], *small_cp, w_cp[1], x_cp[1], w_cp[2], x_cp[2], x_cp[3], *late_cp]:
        c.start()
    bias_v[...] = jnp.where(_iota((T, T), 0) <= _iota((T, T), 1), 0.0, NEG)
    wo_v[pl.ds(D, DP - D), :] = jnp.zeros((DP - D, D), BF16)
    x_cp[0].wait()
    for t in range(NT):
        layernorm(0, t)
    w_cp[0].wait()
    for t in range(5):
        transpose_weight(0, t)
    for p in range(3):
        project_q(0, p)
    for c in [*small_cp, w_cp[1], x_cp[1]]:
        c.wait()
    project_q(0, 3)
    for t in range(5):
        transpose_weight(1, t)
    for p in range(4):
        project_k(0, p)
        layernorm(1, p)
    small_tables()
    for p in range(4):
        project_q(1, p)
    for p in range(3):
        project_k(1, p)
    for c in [w_cp[2], x_cp[2], x_cp[3]]:
        c.wait()
    project_k(1, 3)
    for t in range(5):
        transpose_weight(2, t)
    for s in range(2):
        for p in range(4):
            project_v(s, p)
            layernorm(s + 2, p)
    for s in range(2, NSEG):
        for f in (project_v, project_q, project_k):
            for p in range(4):
                f(s, p)

    blocks = [(s, i, j) for s in range(NSEG) for i in reversed(range(NT)) for j in range(i + 1)]

    def attend(g, true_max, side=()):
        row = _iota((GP, T), 0)
        lane = _iota((GP, T), 1)
        mz_mask = jnp.zeros((GP, T), jnp.bool_)
        for h in range(HG):
            in_row = ((row >= h * DH) & (row < (h + 1) * DH)) | (row == GR + h)
            mz_mask = mz_mask | (in_row & (lane >= h * DH) & (lane < (h + 1) * DH))
        row8 = _iota((8, T), 0)
        numer = gate_v[pl.ds(_aligned(g * 8, 8), 8), :]
        st, run_max, col_max, acc, mem, mz, lim = {}, {}, {}, {}, {}, [None], []

        def scores(n):
            s, i, j = blocks[n]
            kt = _bf(kn_v[s, g, pl.ds(j * T // 2, T // 2), :])
            for h in range(HG):
                parts = [_bf(qs_v[s, g, h, :, pl.ds(i * T, T)]), jnp.zeros((T - 32 - 16 * h, T), BF16)]
                if h:
                    parts.insert(0, jnp.zeros((16 * h, T), BF16))
                t = _dot(kt, jnp.concatenate(parts, axis=0))
                if j == i:
                    t = t + bias_v[...]
                st[n, h] = t
                if true_max:
                    m = jnp.max(t, axis=0, keepdims=True)
                    run_max[h] = m if j == 0 else jnp.maximum(run_max[h], m)
                    col_max[s, i, h] = run_max[h]

        def values(n):
            s, i, j = blocks[n]
            for h in range(HG):
                w = vt_v[s, g, pl.ds(16 * h, 24), pl.ds(j * T, T)]
                if h < HG - 1:
                    w = jnp.concatenate([w[:16], jnp.where(row8 == 5 + h, 1.0, w[16:])], axis=0)
                else:
                    w = jnp.concatenate([jnp.where(row8 == 4, 1.0, w[:8]), w[8:]], axis=0)
                t = st.pop((n, h))
                p = jnp.exp2(t - col_max[s, i, h] if true_max else t)
                a = _dot(w, p.astype(BF16))
                acc[h] = a if j == 0 else acc[h] + a
            if j < i:
                return
            den = jnp.where(row8 < 5, acc[3][:8], acc[2][16:])
            den = jnp.where(row8 == 5, acc[0][16:], jnp.where(row8 == 6, acc[1][16:], den))
            lim[:] = [jnp.minimum(lim[0], den), jnp.maximum(lim[1], den)] if lim else [den, den]
            if s > 0:
                mt = mem[s][:, i * T:(i + 1) * T]
                den = jnp.where(row8 < 4, mt[GR:] + 1e-6, den)
            coef = numer / den

            def spread(lo, mid, hi):
                out = [lo[0], mid[0]]
                for h in range(1, HG):
                    out += [jnp.where(row8 < 2 * h, hi[h - 1], lo[h]), mid[h]]
                return jnp.concatenate(out + [hi[HG - 1]], axis=0)

            cl = [jnp.broadcast_to(coef[r:r + 1], (8, T)) for r in (5, 6, 7, 4)]
            o = spread(*[[acc[h][r:r + 8] for h in range(HG)] for r in (0, 8, 16)]) * spread(cl, cl, cl)
            if s > 0:
                cm = [jnp.broadcast_to(coef[r:r + 1], (8, T)) for r in range(HG)]
                o = o + mt[:GR] * spread(cm, cm, cm)
            ot_v[s, pl.ds(_aligned(g * GR, 8), GR), pl.ds(i * T, T)] = o

        def mem_update(s):
            pk = _phi(_bf(kn_v[s, g]).astype(F32)).astype(BF16)
            va = jnp.concatenate([vt_v[s, g], jnp.ones((GP - GR, L), F32)], axis=0)
            upd = jnp.where(mz_mask, _dot(va, pk), 0.0)
            mz[0] = upd if mz[0] is None else mz[0] + upd

        def mem_read(s):
            mem[s] = _dot(mz[0][:, :GP], _bf(pq_v[s, g]))

        lag = NT + 1 if true_max else LAG
        for n in range(len(blocks) + lag):
            if n < len(blocks):
                scores(n)
                s, k = divmod(n, len(blocks) // NSEG)
                if s < NSEG - 1 and k == 2:
                    mem_update(s)
                if s > 0 and k == 0:
                    mem_read(s)
            if n >= lag:
                values(n - lag)
            for f in side[n * len(side) // len(blocks):(n + 1) * len(side) // len(blocks)]:
                f()
        return lim

    def attend_fast(g, side):
        lo, hi = attend(g, False, side)
        if not (isinstance(g, int) and g == 0):
            lo, hi = jnp.minimum(lim_v[0], lo), jnp.maximum(lim_v[1], hi)
        lim_v[0] = lo
        lim_v[1] = hi

    def route():
        state = {}

        def top2():
            r = _round_bf16(jnp.concatenate([r_v[s] for s in range(NSEG)], axis=1))
            pos = _iota((8, S), 1)
            m1 = jnp.max(r, axis=1, keepdims=True)
            i1 = jnp.min(jnp.where(r == m1, pos, S), axis=1, keepdims=True)
            r2 = jnp.where(pos == i1, -jnp.inf, r)
            m2 = jnp.max(r2, axis=1, keepdims=True)
            i2 = jnp.min(jnp.where((r2 == m2) & (pos != i1), pos, S), axis=1, keepdims=True)
            sub = _iota((8, S), 0)
            onehot = jnp.where(((sub == 0) & (pos == i1)) | ((sub == 1) & (pos == i2)), 1.0, 0.0)
            for s in range(NSEG):
                ot_v[s, pl.ds(D, 8), :] = onehot[:, s * L:(s + 1) * L]
            rs_v[...] = jnp.broadcast_to(
                jax.nn.sigmoid(jnp.where(_iota((8, 1), 0) == 0, m1, m2)), (8, T))
            for c, idx in enumerate((i1, i2)):
                state[c] = jnp.broadcast_to(idx, (8, T)) - _iota((8, T), 1)

        def clear(s):
            ot_v[s, pl.ds(D + 8, DP - D - 8), :] = jnp.zeros((DP - D - 8, L), F32)

        def gather(d):
            n = min(T, D - d)
            both = None
            for c in range(2):
                rel = jnp.concatenate([state[c]] * (n // 16), axis=0)
                col = jnp.zeros((n // 2, T), U32)
                for t in range(S // T):
                    col = jnp.where(rel == t * T,
                                    xn_v[t // NT, pl.ds(d // 2, n // 2), pl.ds(t % NT * T, T)], col)
                col = jnp.sum(_bf(col).astype(F32), axis=1, keepdims=True)
                both = jnp.where(_iota((n, T), 1) == c, col, 0.0 if both is None else both)
            xs_v[:, pl.ds(d, n)] = both.T[:8]
            y_v[:, pl.ds(d, n)] = jnp.zeros((8, n), F32)

        return ([top2] + [partial(clear, s) for s in range(NSEG)]
                + [partial(gather, d) for d in range(0, D, T)])

    def ffn_slice(u):
        cols = pl.ds(_aligned(u * L, L), L)
        acc = {}

        def gate_up(m, d):
            n = min(T, D - d)
            a = _dot(xs_v[:, pl.ds(d, n)], (wg_v, wu_v)[m][pl.ds(d, n), cols])
            acc[m] = acc[m] + a if d else a

        def down(d):
            n = min(T, D - d)
            if d == 0:
                acc[2] = acc[0] * jax.nn.sigmoid(acc[0]) * acc[1]
            y_v[:, pl.ds(d, n)] += jax.lax.dot_general(
                acc[2], wd_v[pl.ds(d, n), cols], (((1,), (1,)), ((), ())), preferred_element_type=F32)

        return ([partial(gate_up, m, d) for m in range(2) for d in range(0, D, T)] + [lambda: None]
                + [partial(down, d) for d in range(0, D, T)])

    def output_weights(t):
        if (t + 1) * T == DP:
            y = y_v[...] * rs_v[:, pl.ds(0, 1)]
            wo_v[pl.ds(D, 16), :] = jnp.concatenate([y, jnp.zeros((8, D), F32)], axis=0).astype(BF16)
        wot_v[:, pl.ds(t * T, T)] = pltpu.bitcast(wo_v[pl.ds(t * T, T), :].T, U32)

    attend_fast(0, route())
    for c in late_cp:
        c.wait()

    def middle(it, carry):
        side = ffn_slice(3 * it) + ffn_slice(3 * it + 1) + ffn_slice(3 * it + 2)
        attend_fast(2 * it + 1, side[:len(side) // 2])
        attend_fast(2 * it + 2, side[len(side) // 2:])
        return carry

    jax.lax.fori_loop(0, (NG - 2) // 2, middle, 0)
    attend_fast(NG - 1, [partial(output_weights, t) for t in range(DP // T)])

    safe = (_iota((8, T), 0) < 4) | ((lim_v[0] >= SAFE_LO) & (lim_v[1] <= SAFE_HI))

    @pl.when(jnp.min(jnp.where(safe, 1, 0)) == 0)
    def _():
        jax.lax.fori_loop(0, NG, lambda g, c: (attend(g, True), c)[1], 0)

    def out_copy(s):
        return pltpu.make_async_copy(out_v.at[s], out_hbm.at[:, pl.ds(s * L, L)], out_sem.at[s])

    for s in range(NSEG):
        att = _dot(_bf(wot_v[...]), ot_v[s].astype(BF16))
        out_v[s] = (x_v[s].astype(F32) + att + _bf(xn_v[s]).astype(F32)).astype(BF16)
        out_copy(s).start()
    for s in range(NSEG):
        out_copy(s).wait()


@jax.jit
def pallas_parallel_sum__memory_aug_infini_attn__moe_arch_mod__prompt_kernel(
    A_x: jax.Array,
    A_wq: jax.Array,
    A_wk: jax.Array,
    A_wv: jax.Array,
    A_wo: jax.Array,
    A_beta: jax.Array,
    B_x: jax.Array,
    B_w_r: jax.Array,
    B_w_gate: jax.Array,
    B_w_up: jax.Array,
    B_w_down: jax.Array,
):
    del B_x
    assert A_x.shape == (1, S, D) and B_w_gate.shape == (D, FF)
    hbm = pl.BlockSpec(memory_space=pl.ANY)
    out_t = pl.pallas_call(
        _kernel,
        out_shape=jax.ShapeDtypeStruct((D, S), BF16),
        in_specs=[hbm] * 10,
        out_specs=hbm,
        scratch_shapes=[
            pltpu.VMEM((D,), BF16),
            pltpu.VMEM((H,), BF16),
            pltpu.VMEM((NSEG, D, L), BF16),
            pltpu.VMEM((3, D, D), BF16),
            pltpu.VMEM((DP, D), BF16),
            pltpu.VMEM((3 * D // 2 + 8, D), U32),
            pltpu.VMEM((D // 2, DP), U32),
            pltpu.VMEM((NSEG, D // 2, L), U32),
            pltpu.VMEM((NSEG, NG, HG, 16, L), U32),
            pltpu.VMEM((NSEG, NG, GP // 2, L), U32),
            pltpu.VMEM((NSEG, NG, L // 2, T), U32),
            pltpu.VMEM((NSEG, NG, GR, L), F32),
            pltpu.VMEM((NSEG, DP, L), F32),
            pltpu.VMEM((NSEG, 8, L), F32),
            pltpu.VMEM((NG * 8, T), F32),
            pltpu.VMEM((T, T), F32),
            pltpu.VMEM((2, 8, T), F32),
            pltpu.VMEM((8, D), F32),
            pltpu.VMEM((8, D), F32),
            pltpu.VMEM((8, T), F32),
            pltpu.VMEM((D, FF), BF16),
            pltpu.VMEM((D, FF), BF16),
            pltpu.VMEM((D, FF), BF16),
            pltpu.VMEM((NSEG, D, L), BF16),
            pltpu.SemaphoreType.DMA((NSEG + 9,)),
            pltpu.SemaphoreType.DMA((NSEG,)),
        ],
        compiler_params=pltpu.CompilerParams(vmem_limit_bytes=100 * 2 ** 20),
        name="infini_mod",
    )(B_w_r, A_beta, A_x[0].T, A_wq, A_wk, A_wv, A_wo, B_w_gate, B_w_up, B_w_down.T)
    return out_t.T[None]
```

```python
import math
from functools import partial

import jax
import jax.numpy as jnp
import jax.experimental.pallas as pl
import jax.experimental.pallas.tpu as pltpu

D = 576
S = 2048
H = 32
DH = D // H
NSEG = 4
L = S // NSEG
FF = 4608
HG = 4
NG = H // HG
GR = HG * DH
GP = 80
T = 128
NT = L // T
CH = 2 * GR
DP = 640
FT = FF // T // (NG - 2)

F32 = jnp.float32
BF16 = jnp.bfloat16
U32 = jnp.uint32
QSCALE = (DH ** -0.5) * math.log2(math.e)
NEG = -1e30
SAFE_LO, SAFE_HI = 2.0 ** -30, 2.0 ** 30
LAG = 2
PRI = 0
NODMA = 0
MR = 1
MU = 5
PADN = 10
UNR = 1
FCH = 2


def _iota(shape, dim):
    return jax.lax.broadcasted_iota(jnp.int32, shape, dim)


def _round_bf16(t):
    return t.astype(BF16).astype(F32)


def _pack(t):
    return pltpu.bitcast(t.astype(BF16), U32)


def _bf(t):
    return pltpu.bitcast(t, BF16)


def _phi(t):
    return jnp.where(t > 0, t + 1.0, jnp.exp(t))


def _dot(a, b):
    return jax.lax.dot_general(a, b, (((1,), (0,)), ((), ())), preferred_element_type=F32)


def _aligned(i, n):
    return i if isinstance(i, int) else pl.multiple_of(i, n)


def _kernel(wr_hbm, beta_hbm, x_hbm, wq_hbm, wk_hbm, wv_hbm, wo_hbm, wg_hbm, wu_hbm, wd_hbm,
            out_hbm,
            wr_v, beta_v, x_v, wraw_v, wo_v, wt_v, wot_v, xn_v, qs_v, pq_v, kn_v, vt_v, ot_v,
            r_v, gate_v, bias_v, lim_v, xs_v, y_v, rs_v, wg_v, wu_v, wd_v, out_v, zero_s,
            in_sem, out_sem):
    x_cp = [pltpu.make_async_copy(x_hbm.at[:, pl.ds(s * L, L)], x_v.at[s], in_sem.at[s])
            for s in range(NSEG)]
    w_cp = [pltpu.make_async_copy(w, wraw_v.at[i], in_sem.at[NSEG + i])
            for i, w in enumerate((wq_hbm, wk_hbm, wv_hbm))]
    late_cp = [pltpu.make_async_copy(src, dst, in_sem.at[NSEG + 3 + i]) for i, (src, dst) in enumerate(
        ((wo_hbm, wo_v.at[pl.ds(0, D)]), (wg_hbm, wg_v), (wu_hbm, wu_v), (wd_hbm, wd_v)))]
    small_cp = [pltpu.make_async_copy(wr_hbm, wr_v, in_sem.at[NSEG + 7]),
                pltpu.make_async_copy(beta_hbm, beta_v, in_sem.at[NSEG + 8])]

    def layernorm(s, t):
        cols = pl.ds(t * T, T)
        shift = jnp.broadcast_to(x_v[s, pl.ds(0, 16), cols].astype(F32)[:1], (16, T))
        s1 = s2 = None
        for d in range(0, D, 16):
            xc = x_v[s, pl.ds(d, 16), cols].astype(F32) - shift
            s1, s2 = (xc, xc * xc) if d == 0 else (s1 + xc, s2 + xc * xc)
        m = jnp.sum(s1, axis=0, keepdims=True) * (1.0 / D)
        v = jnp.maximum(jnp.sum(s2, axis=0, keepdims=True) * (1.0 / D) - m * m, 0.0)
        m = jnp.broadcast_to(_round_bf16(m + shift[:1]), (16, T))
        inv = jnp.broadcast_to(1.0 / _round_bf16(jnp.sqrt(_round_bf16(_round_bf16(v) + 1e-5))), (16, T))
        again = s + zero_s[0]
        for d in range(0, D, 16):
            x = x_v[again, pl.ds(d, 16), cols].astype(F32)
            xn_v[s, pl.ds(d // 2, 8), cols] = _pack(_round_bf16(x - m) * inv)

    def transpose_weight(i, t):
        n = min(T, D - t * T)
        wt_v[pl.ds((i * D + t * T) // 2, n // 2), :] = pltpu.bitcast(
            wraw_v[i, :, pl.ds(t * T, n)].T, U32)

    def proj(s, row, n):
        return _dot(_bf(wt_v[pl.ds(row // 2, n // 2), :]), _bf(xn_v[s]))

    def project_q(s, p):
        zpad = jnp.zeros((GP - GR, L), F32)
        row32 = _iota((32, L), 0)
        q = proj(s, p * CH, CH)
        pq = _phi(q) if s else None
        q = q * QSCALE
        for j in range(2):
            rows = slice(j * GR, (j + 1) * GR)
            qg = jnp.concatenate([q[rows], zpad], axis=0)
            for h in range(HG):
                keep = (row32 >= 2 * h) & (row32 < 2 * h + DH)
                qs_v[s, 2 * p + j, h] = _pack(jnp.where(keep, qg[16 * h:16 * h + 32], 0.0))
            if s:
                pq_v[s, 2 * p + j] = _pack(jnp.concatenate([pq[rows], zpad], axis=0))

    def project_k(s, p):
        k = proj(s, D + p * CH, CH)
        for j in range(2):
            kg = jnp.concatenate([k[j * GR:(j + 1) * GR], jnp.zeros((T - GR, L), F32)], axis=0)
            kn_v[s, 2 * p + j] = pltpu.bitcast(kg.astype(BF16).T, U32)

    def project_v(s, p):
        extra = 16 if p == NG // 2 - 1 else 0
        v = proj(s, 2 * D + p * CH, CH + extra)
        for j in range(2):
            vt_v[s, 2 * p + j] = v[j * GR:(j + 1) * GR]
        if extra:
            r_v[s] = v[CH:CH + 8]

    def small_tables():
        wt_v[pl.ds(3 * D // 2, 8), :] = _pack(
            jnp.broadcast_to(wr_v[...].astype(F32).reshape(1, D), (16, D)))
        sg = jax.nn.sigmoid(beta_v[...].astype(F32).reshape(1, H))
        trow = _iota((NG * 8, H), 0)
        head = (trow >> 3) * HG + ((trow + jnp.where((trow & 4) != 0, 3, 0)) & 3)
        gcol = jnp.sum(jnp.where(_iota((NG * 8, H), 1) == head,
                                 jnp.broadcast_to(sg, (NG * 8, H)), 0.0), axis=1, keepdims=True)
        gcol = jnp.where((_iota((NG * 8, 1), 0) & 4) != 0, 1.0 - gcol, gcol)
        gate_v[...] = jnp.broadcast_to(gcol, (NG * 8, T))

    for c in [x_cp[0], *w_cp, *small_cp, *x_cp[1:], *late_cp]:
        c.start()
    zero_s[0] = 0
    bias_v[...] = jnp.where(_iota((T, T), 0) <= _iota((T, T), 1), 0.0, NEG)
    wo_v[pl.ds(D, DP - D), :] = jnp.zeros((DP - D, D), BF16)
    for s in range(NSEG):
        ot_v[s, pl.ds(D + 8, DP - D - 8), :] = jnp.zeros((DP - D - 8, L), F32)
    x_cp[0].wait()
    for t in range(NT):
        layernorm(0, t)
    w_cp[0].wait()
    for t in range(5):
        transpose_weight(0, t)
    for p in range(3):
        project_q(0, p)
    w_cp[1].wait()
    project_q(0, 3)
    for t in range(5):
        transpose_weight(1, t)
    for p in range(3):
        project_k(0, p)
    for c in [w_cp[2], *small_cp, x_cp[1]]:
        c.wait()
    project_k(0, 3)
    for t in range(5):
        transpose_weight(2, t)
    small_tables()
    for p in range(4):
        project_v(0, p)
        layernorm(1, p)
    for f in (project_k, project_q):
        for p in range(4):
            f(1, p)
    for c in x_cp[2:]:
        c.wait()
    for s in range(1, NSEG):
        for p in range(4):
            project_v(s, p)
            if s + 1 < NSEG:
                layernorm(s + 1, p)
        for f in (project_k, project_q):
            for p in range(4):
                if s > 1:
                    f(s, p)

    tiles = [(s, i, j) for s in range(NSEG) for i in reversed(range(NT)) for j in range(i + 1)]

    def attend(groups, true_max, side=()):
        blocks = [(k, *t) for k in range(len(groups)) for t in tiles]
        row = _iota((GP, T), 0)
        lane = _iota((GP, T), 1)
        mz_mask = jnp.zeros((GP, T), jnp.bool_)
        for h in range(HG):
            in_row = ((row >= h * DH) & (row < (h + 1) * DH)) | (row == GR + h)
            mz_mask = mz_mask | (in_row & (lane >= h * DH) & (lane < (h + 1) * DH))
        row8 = _iota((8, T), 0)
        st, col_max, acc, mem, mz, lim = {}, {}, {}, {}, {}, []

        def scores(n):
            k, s, i, j = blocks[n]
            kt = _bf(kn_v[s, groups[k], pl.ds(j * T // 2, T // 2), :])
            for h in range(HG):
                parts = [_bf(qs_v[s, groups[k], h, :, pl.ds(i * T, T)]),
                         jnp.zeros((T - 32 - 16 * h, T), BF16)]
                if h:
                    parts.insert(0, jnp.zeros((16 * h, T), BF16))
                t = _dot(kt, jnp.concatenate(parts, axis=0))
                if j == i:
                    t = t + bias_v[...]
                st[n, h] = t
                if true_max:
                    m = jnp.max(t, axis=0, keepdims=True)
                    col_max[k, s, i, h] = jnp.maximum(col_max[k, s, i, h], m) if j else m

        def values(n):
            k, s, i, j = blocks[n]
            g = groups[k]
            for h in range(HG):
                w = vt_v[s, g, pl.ds(16 * h, 24), pl.ds(j * T, T)]
                if h < HG - 1:
                    w = jnp.concatenate([w[:16], jnp.where(row8 == 5 + h, 1.0, w[16:])], axis=0)
                else:
                    w = jnp.concatenate([jnp.where(row8 == 4, 1.0, w[:8]), w[8:]], axis=0)
                t = st.pop((n, h))
                p = jnp.exp2(t - col_max[k, s, i, h] if true_max else t)
                a = _dot(w, p.astype(BF16))
                acc[h] = acc[h] + a if j else a
            if j < i:
                return
            den = jnp.where(row8 < 5, acc[3][:8], acc[2][16:])
            den = jnp.where(row8 == 5, acc[0][16:], jnp.where(row8 == 6, acc[1][16:], den))
            lim[:] = [jnp.minimum(lim[0], den), jnp.maximum(lim[1], den)] if lim else [den, den]
            if s > 0:
                mt = mem[k, s][:, i * T:(i + 1) * T]
                den = jnp.where(row8 < 4, mt[GR:] + 1e-6, den)
            coef = gate_v[pl.ds(_aligned(g * 8, 8), 8), :] / den

            def spread(lo, mid, hi):
                out = [lo[0], mid[0]]
                for h in range(1, HG):
                    out += [jnp.where(row8 < 2 * h, hi[h - 1], lo[h]), mid[h]]
                return jnp.concatenate(out + [hi[HG - 1]], axis=0)

            cl = [jnp.broadcast_to(coef[r:r + 1], (8, T)) for r in (5, 6, 7, 4)]
            o = spread(*[[acc[h][r:r + 8] for h in range(HG)] for r in (0, 8, 16)]) * spread(cl, cl, cl)
            if s > 0:
                cm = [jnp.broadcast_to(coef[r:r + 1], (8, T)) for r in range(HG)]
                o = o + mt[:GR] * spread(cm, cm, cm)
            ot_v[s, pl.ds(_aligned(g * GR, 8), GR), pl.ds(i * T, T)] = o

        def mem_update(k, s):
            pk = _phi(_bf(kn_v[s, groups[k]]).astype(F32)).astype(BF16)
            va = jnp.concatenate([vt_v[s, groups[k]], jnp.ones((GP - GR, L), F32)], axis=0)
            upd = jnp.where(mz_mask, _dot(va, pk), 0.0)
            mz[k] = mz[k] + upd if s else upd

        def mem_read(k, s):
            mem[k, s] = _dot(mz[k][:, :GP], _bf(pq_v[s, groups[k]]))

        lag = NT + 1 if true_max else LAG
        for n in range(len(blocks) + lag):
            if n < len(blocks):
                scores(n)
                k, s = blocks[n][:2]
                pos = n % (len(tiles) // NSEG)
                if s > 0 and pos == MR:
                    mem_read(k, s)
                if s < NSEG - 1 and pos == MU:
                    mem_update(k, s)
            if n >= lag:
                values(n - lag)
            for f in side[n * len(side) // len(blocks):(n + 1) * len(side) // len(blocks)]:
                f()
        return lim

    def route():
        state = {}

        def top2():
            r = _round_bf16(jnp.concatenate([r_v[s] for s in range(NSEG)], axis=1))
            pos = _iota((8, S), 1)
            m1 = jnp.max(r, axis=1, keepdims=True)
            i1 = jnp.min(jnp.where(r == m1, pos, S), axis=1, keepdims=True)
            r2 = jnp.where(pos == i1, -jnp.inf, r)
            m2 = jnp.max(r2, axis=1, keepdims=True)
            i2 = jnp.min(jnp.where((r2 == m2) & (pos != i1), pos, S), axis=1, keepdims=True)
            sub = _iota((8, S), 0)
            onehot = jnp.where(((sub == 0) & (pos == i1)) | ((sub == 1) & (pos == i2)), 1.0, 0.0)
            for s in range(NSEG):
                ot_v[s, pl.ds(D, 8), :] = onehot[:, s * L:(s + 1) * L]
            rs_v[...] = jnp.broadcast_to(
                jax.nn.sigmoid(jnp.where(_iota((8, 1), 0) == 0, m1, m2)), (8, T))
            for c, idx in enumerate((i1, i2)):
                state[c] = jnp.broadcast_to(idx, (8, T)) - _iota((8, T), 1)

        def gather(d):
            n = min(T, D - d)
            both = None
            for c in range(2):
                rel = jnp.concatenate([state[c]] * (n // 16), axis=0)
                col = jnp.zeros((n // 2, T), U32)
                for t in range(S // T):
                    col = jnp.where(rel == t * T,
                                    xn_v[t // NT, pl.ds(d // 2, n // 2), pl.ds(t % NT * T, T)], col)
                col = jnp.sum(_bf(col).astype(F32), axis=1, keepdims=True)
                both = jnp.where(_iota((n, T), 1) == c, col, 0.0 if both is None else both)
            xs_v[:, pl.ds(d, n)] = both.T[:8]
            y_v[:, pl.ds(d, n)] = jnp.zeros((8, n), F32)

        return [top2] + [partial(gather, d) for d in range(0, D, T)]

    def ffn_slice(u):
        cols = pl.ds(_aligned(u * L, L), L)
        acc = {}

        def gate_up(m, d):
            n = min(T, D - d)
            a = _dot(xs_v[:, pl.ds(d, n)], (wg_v, wu_v)[m][pl.ds(d, n), cols])
            acc[m] = acc[m] + a if d else a

        def down(d):
            n = min(T, D - d)
            if d == 0:
                acc[2] = acc[0] * jax.nn.sigmoid(acc[0]) * acc[1]
            y_v[:, pl.ds(d, n)] += jax.lax.dot_general(
                acc[2], wd_v[pl.ds(d, n), cols], (((1,), (1,)), ((), ())), preferred_element_type=F32)

        return ([partial(gate_up, m, d) for m in range(2) for d in range(0, D, T)] + [lambda: None]
                + [partial(down, d) for d in range(0, D, T)])

    def output_weights(t):
        if (t + 1) * T == DP:
            y = y_v[...] * rs_v[:, pl.ds(0, 1)]
            wo_v[pl.ds(D, 16), :] = jnp.concatenate([y, jnp.zeros((8, D), F32)], axis=0).astype(BF16)
        wot_v[:, pl.ds(t * T, T)] = pltpu.bitcast(wo_v[pl.ds(t * T, T), :].T, U32)

    def output():
        pieces = [(s, 0, D) for s in range(NSEG - 1)]
        pieces += [(NSEG - 1, r, n) for r, n in ((0, 288), (288, 192), (480, 96))]
        out_cp = []
        for i, (s, r, n) in enumerate(pieces):
            rows, half = pl.ds(r, n), pl.ds(r // 2, n // 2)
            att = _dot(_bf(wot_v[half, :]), ot_v[s].astype(BF16))
            out_v[s, rows, :] = (
                x_v[s, rows, :].astype(F32) + att + _bf(xn_v[s, half, :]).astype(F32)).astype(BF16)
            out_cp.append(pltpu.make_async_copy(
                out_v.at[s, rows, :], out_hbm.at[rows, pl.ds(s * L, L)], out_sem.at[i]))
            out_cp[-1].start()
        return out_cp

    lim_v[0], lim_v[1] = attend([0], False, route())
    for c in late_cp:
        c.wait()
    side = [f for u in range(FF // L) for f in ffn_slice(u)]
    side += [partial(output_weights, t) for t in range(DP // T)] + [lambda: None] * PADN
    lo, hi = attend(list(range(1, NG)), False, side)
    safe = (_iota((8, T), 0) < 4) | ((jnp.minimum(lim_v[0], lo) >= SAFE_LO)
                                     & (jnp.maximum(lim_v[1], hi) <= SAFE_HI))
    unsafe = jnp.min(jnp.where(safe, 1, 0)) == 0
    for c in output():
        c.wait()

    @pl.when(unsafe)
    def _():
        jax.lax.fori_loop(0, NG, lambda g, c: (attend([g], True), c)[1], 0)
        for c in output():
            c.wait()


@jax.jit
def pallas_parallel_sum__memory_aug_infini_attn__moe_arch_mod__prompt_kernel(
    A_x: jax.Array,
    A_wq: jax.Array,
    A_wk: jax.Array,
    A_wv: jax.Array,
    A_wo: jax.Array,
    A_beta: jax.Array,
    B_x: jax.Array,
    B_w_r: jax.Array,
    B_w_gate: jax.Array,
    B_w_up: jax.Array,
    B_w_down: jax.Array,
):
    del B_x
    assert A_x.shape == (1, S, D) and B_w_gate.shape == (D, FF)
    hbm = pl.BlockSpec(memory_space=pl.ANY)
    out_t = pl.pallas_call(
        _kernel,
        out_shape=jax.ShapeDtypeStruct((D, S), BF16),
        in_specs=[hbm] * 10,
        out_specs=hbm,
        scratch_shapes=[
            pltpu.VMEM((D,), BF16),
            pltpu.VMEM((H,), BF16),
            pltpu.VMEM((NSEG, D, L), BF16),
            pltpu.VMEM((3, D, D), BF16),
            pltpu.VMEM((DP, D), BF16),
            pltpu.VMEM((3 * D // 2 + 8, D), U32),
            pltpu.VMEM((D // 2, DP), U32),
            pltpu.VMEM((NSEG, D // 2, L), U32),
            pltpu.VMEM((NSEG, NG, HG, 16, L), U32),
            pltpu.VMEM((NSEG, NG, GP // 2, L), U32),
            pltpu.VMEM((NSEG, NG, L // 2, T), U32),
            pltpu.VMEM((NSEG, NG, GR, L), F32),
            pltpu.VMEM((NSEG, DP, L), F32),
            pltpu.VMEM((NSEG, 8, L), F32),
            pltpu.VMEM((NG * 8, T), F32),
            pltpu.VMEM((T, T), F32),
            pltpu.VMEM((2, 8, T), F32),
            pltpu.VMEM((8, D), F32),
            pltpu.VMEM((8, D), F32),
            pltpu.VMEM((8, T), F32),
            pltpu.VMEM((D, FF), BF16),
            pltpu.VMEM((D, FF), BF16),
            pltpu.VMEM((D, FF), BF16),
            pltpu.VMEM((NSEG, D, L), BF16),
            pltpu.SMEM((1,), jnp.int32),
            pltpu.SemaphoreType.DMA((NSEG + 9,)),
            pltpu.SemaphoreType.DMA((NSEG + 2,)),
        ],
        compiler_params=pltpu.CompilerParams(vmem_limit_bytes=100 * 2 ** 20),
        name="infini_mod",
    )(B_w_r, A_beta, A_x[0].T, A_wq, A_wk, A_wv, A_wo, B_w_gate, B_w_up, B_w_down.T)
    return out_t.T[None]
```

```python
import math
from functools import partial

import jax
import jax.numpy as jnp
import jax.experimental.pallas as pl
import jax.experimental.pallas.tpu as pltpu

D = 576
S = 2048
H = 32
DH = D // H
NSEG = 4
L = S // NSEG
FF = 4608
HG = 4
NG = H // HG
GR = HG * DH
GP = 80
T = 128
QT = T // HG
NT = L // T
CH = 2 * GR
NCH = D // CH
DP = 640
WO = 3 * D // 2 + 8

F32 = jnp.float32
BF16 = jnp.bfloat16
U32 = jnp.uint32
QSCALE = (DH ** -0.5) * math.log2(math.e)
NEG = -1e30
SAFE_LO, SAFE_HI = 2.0 ** -30, 2.0 ** 30
LAG = 3
MEM_READ_STEP = 3
MEM_UPDATE_STEP = 6
FFN_FIRST_STEP = 50
FFN_STEPS = (0, 1, 2, 4, 5, 7)


def _iota(shape, dim):
    return jax.lax.broadcasted_iota(jnp.int32, shape, dim)


def _round_bf16(t):
    return t.astype(BF16).astype(F32)


def _pack(t):
    return pltpu.bitcast(t.astype(BF16), U32)


def _bf(t):
    return pltpu.bitcast(t, BF16)


def _split(t):
    return [pltpu.unpack_elementwise(t, index=i, packed_dtype=BF16, unpacked_dtype=F32)
            for i in range(2)]


def _join(ts):
    return pltpu.pack_elementwise(ts, packed_dtype=BF16)


def _phi(t):
    return jnp.where(t > 0, t + 1.0, jnp.exp(t))


def _dot(a, b):
    return jax.lax.dot_general(a, b, (((1,), (0,)), ((), ())), preferred_element_type=F32)


def _dot_nt(a, b):
    return jax.lax.dot_general(a, b, (((1,), (1,)), ((), ())), preferred_element_type=F32)


def _aligned(i, n):
    return i if isinstance(i, int) else pl.multiple_of(i, n)


def _kernel(wr_hbm, beta_hbm, x_hbm, wq_hbm, wk_hbm, wv_hbm, wo_hbm, wg_hbm, wu_hbm, wd_hbm,
            out_hbm,
            wr_v, beta_v, x_v, wraw_v, wo_v, wt_v, xn_v, qs_v, qx_v, pq_v, kn_v, vt_v, acc_v,
            mem_v, ot_v, r_v, gate_v, bias_v, xs_v, y_v, rs_v, wg_v, wu_v, wd_v, out_v,
            in_sem, out_sem):
    x_cp = [pltpu.make_async_copy(x_hbm.at[:, pl.ds(s * L, L)], x_v.at[s], in_sem.at[s])
            for s in range(NSEG)]
    wq_cp, wk_cp, wv_cp, wo_cp, *more_cp = [
        pltpu.make_async_copy(src, dst, in_sem.at[NSEG + i]) for i, (src, dst) in enumerate((
            (wq_hbm, wraw_v.at[0]), (wk_hbm, wraw_v.at[1]), (wv_hbm, wraw_v.at[2]),
            (wo_hbm, wo_v.at[pl.ds(0, D)]), (wr_hbm, wr_v), (beta_hbm, beta_v),
            (wg_hbm, wg_v), (wu_hbm, wu_v), (wd_hbm, wd_v)))]
    small_cp, ffn_cp = more_cp[:2], more_cp[2:]
    for c in [x_cp[0], wv_cp, *small_cp, wq_cp, wk_cp, *x_cp[1:], wo_cp, *ffn_cp]:
        c.start()

    zero = jnp.min(_iota((8, T), 1))
    zeros = _iota((8, T), 1) * zero
    marks = []

    def marker(*values):
        out = pltpu.bitcast(values[0], jnp.int32)
        for t in values[1:]:
            out = out | pltpu.bitcast(t, jnp.int32)
        return out & zeros

    def tied(t, mark):
        head = pltpu.bitcast(pltpu.bitcast(t[:8, :T], jnp.int32) | mark, t.dtype)
        return jnp.concatenate([jnp.concatenate([head, t[:8, T:]], axis=1), t[8:]], axis=0)

    def layernorm(s, t):
        cols = pl.ds(t * T, T)
        shift = jnp.broadcast_to(x_v[s, pl.ds(0, 16), cols].astype(F32)[:1], (16, T))
        for d in range(0, D, 16):
            xc = x_v[s, pl.ds(d, 16), cols].astype(F32) - shift
            s1, s2 = (s1 + xc, s2 + xc * xc) if d else (xc, xc * xc)
        m = jnp.sum(s1, axis=0, keepdims=True) * (1.0 / D)
        v = jnp.maximum(jnp.sum(s2, axis=0, keepdims=True) * (1.0 / D) - m * m, 0.0)
        m = jnp.broadcast_to(_round_bf16(m + shift[:1]), (8, T))
        inv = jnp.broadcast_to(
            1.0 / _round_bf16(jnp.sqrt(_round_bf16(_round_bf16(v) + 1e-5))), (8, T))
        for d in range(0, D, 16):
            x = _split(pltpu.bitcast(x_v[s + zero, pl.ds(d, 16), cols], U32))
            x = _split(_join([u - m for u in x]))
            xn_v[s, pl.ds(d // 2, 8), cols] = _join([u * inv for u in x])
        return marker(xn_v[s + zero, :8, cols])

    def transpose_weight(i):
        for c in range(0, D, T):
            n = min(T, D - c)
            wt_v[pl.ds((i * D + c) // 2, n // 2), pl.ds(0, D)] = pltpu.bitcast(
                wraw_v[i, :, pl.ds(c, n)].T, U32)

    def transpose_wo(c):
        wt_v[pl.ds(WO, D // 2), pl.ds(c, T)] = pltpu.bitcast(wo_v[pl.ds(c, T), :].T, U32)

    def proj(s, row, n):
        w = wt_v[pl.ds(row if not isinstance(row, int) else row // 2, n // 2), pl.ds(0, D)]
        mark = marks.pop(0) if len(marks) > 1 else None
        return _dot(_bf(w if mark is None else tied(w, mark)), _bf(xn_v[s]))

    def project_q(s, p):
        zpad = jnp.zeros((GP - GR, L), F32)
        row32 = _iota((32, L), 0)
        slot = _iota((16, T), 1) >> 5
        q = proj(s, p * CH, CH)
        for j in range(2):
            g = 2 * p + j
            qg = q[j * GR:(j + 1) * GR]
            if s:
                pq_v[s, g] = _pack(jnp.concatenate([_phi(qg), zpad], axis=0))
            qg = jnp.concatenate([qg * QSCALE, zpad], axis=0)
            qh = [_pack(jnp.where((row32 >= 2 * h) & (row32 < 2 * h + DH), qg[16 * h:16 * h + 32], 0.0))
                  for h in range(HG)]
            for t in range(0, L, T):
                cols = pl.ds(t, T)
                rot = [pltpu.roll(w[:, t:t + T], h * QT, 1) if h else w[:, t:t + T]
                       for h, w in enumerate(qh)]
                for h in range(HG):
                    qs_v[s, g, h, :, cols] = rot[h]
                    qx_v[s, g, pl.ds(16 * (h // 2 + h % 2 * 2), 16), cols] = jnp.where(
                        ((slot - h) & 3) >= 2, rot[h], 0)
                for c in (1, 3):
                    ws = [jnp.where(slot == (c + h) % HG, rot[h], 0) for h in range(HG)]
                    qx_v[s, g, pl.ds(44 + 20 * c, 40), cols] = jnp.concatenate(
                        [ws[0][:8], *[a[8:] | b[:8] for a, b in zip(ws, ws[1:])], ws[-1][8:]], axis=0)
        marks.append(marker(qs_v[s + zero, g, 0, :8, :T], qx_v[s + zero, g, :8, :T],
                            *([pq_v[s + zero, g, :8, :T]] if s else [])))

    def project_k(s, p):
        k = proj(s, D + p * CH, CH)
        for j in range(2):
            kg = jnp.concatenate([k[j * GR:(j + 1) * GR], jnp.zeros((T - GR, L), F32)], axis=0)
            kn_v[s, 2 * p + j] = pltpu.bitcast(kg.astype(BF16).T, U32)
        marks.append(marker(kn_v[s + zero, 2 * p, :8, :]))

    def project_v(s, p):
        extra = 16 if p == NCH - 1 else 0
        row = 2 * D + p * CH
        if extra and s == NSEG - 1:
            row = pl.multiple_of(row // 2 + 8 * zero, 8)
        v = proj(s, row, CH + extra)
        for j in range(2):
            vt_v[s, 2 * p + j] = v[j * GR:(j + 1) * GR]
        if extra:
            r_v[s] = v[CH:CH + 8]
        marks.append(None)

    def project(f, s, ps=range(NCH)):
        return [partial(f, s, p) for p in ps]

    def run(dots, norm=None):
        for i, f in enumerate(dots):
            f()
            for t in range(i * NT // len(dots), (i + 1) * NT // len(dots)) if norm else ():
                mark = layernorm(norm, t)
                marks[-1] = mark if marks[-1] is None else marks[-1] | mark

    def small_tables():
        wt_v[pl.ds(3 * D // 2, 8), pl.ds(0, D)] = _pack(
            jnp.broadcast_to(wr_v[...].astype(F32).reshape(1, D), (16, D)))
        sg = jax.nn.sigmoid(beta_v[...].astype(F32).reshape(1, H))
        row = _iota((NG * 8, H), 0)
        head = (row >> 3) * HG + ((row + jnp.where((row & 4) != 0, 3, 0)) & 3)
        gate = jnp.sum(jnp.where(_iota((NG * 8, H), 1) == head,
                                 jnp.broadcast_to(sg, (NG * 8, H)), 0.0), axis=1, keepdims=True)
        gate = jnp.where((_iota((NG * 8, 1), 0) & 4) != 0, 1.0 - gate, gate)
        gate_v[...] = jnp.broadcast_to(gate, (NG * 8, T))

    def top2():
        r = _round_bf16(jnp.concatenate([r_v[s] for s in range(NSEG)], axis=1))
        pos = _iota((8, S), 1)
        m1 = jnp.max(r, axis=1, keepdims=True)
        i1 = jnp.min(jnp.where(r == m1, pos, S), axis=1, keepdims=True)
        r2 = jnp.where(pos == i1, -jnp.inf, r)
        m2 = jnp.max(r2, axis=1, keepdims=True)
        i2 = jnp.min(jnp.where((r2 == m2) & (pos != i1), pos, S), axis=1, keepdims=True)
        sub = _iota((8, S), 0)
        onehot = jnp.where(((sub == 0) & (pos == i1)) | ((sub == 1) & (pos == i2)), 1.0, 0.0)
        for s in range(NSEG):
            ot_v[s, pl.ds(D, 8), :] = onehot[:, s * L:(s + 1) * L]
        rs_v[...] = jnp.broadcast_to(
            jax.nn.sigmoid(jnp.where(_iota((8, 1), 0) == 0, m1, m2)), (8, T))
        return [jnp.clip(jnp.min(i), 0, S - 1) for i in (i1, i2)]

    def gather(tokens, d):
        n = min(L, D - d)
        for c, tok in enumerate(tokens):
            tile = xn_v[tok >> 9, pl.ds(d // 2, n // 2), pl.ds(pl.multiple_of(tok & (L - T), T), T)]
            pick = (_iota((8, T), 0) == c) & (_iota((8, T), 1) == (tok & (T - 1)))
            row = _dot_nt(jnp.where(pick, 1.0, 0.0), _bf(tile))
            rows = row + rows if c else row
        xs_v[:, pl.ds(d, n)] = rows
        y_v[:, pl.ds(d, n)] = jnp.zeros((8, n), F32)

    def ffn_steps(c):
        cols = pl.ds(c, L)
        acc = {}

        def gate_up(m, d):
            rows = pl.ds(d, min(T, D - d))
            a = _dot(xs_v[:, rows], (wg_v, wu_v)[m][rows, cols])
            acc[m] = a + acc[m] if d else a

        def down(d):
            rows = pl.ds(d, min(T, D - d))
            if d == 0:
                acc[2] = acc[0] * jax.nn.sigmoid(acc[0]) * acc[1]
            y_v[:, rows] += _dot_nt(acc[2], wd_v[rows, cols])

        return ([partial(gate_up, m, d) for m in range(2) for d in range(0, D, T)]
                + [partial(down, d) for d in range(0, D, T)])

    def ffn_wait():
        for c in ffn_cp:
            c.wait()

    def ffn_done():
        y = y_v[...] * rs_v[:, pl.ds(0, 1)]
        wo_v[pl.ds(D, 16), :] = jnp.concatenate([y, jnp.zeros((8, D), F32)], axis=0).astype(BF16)
        transpose_wo(DP - T)

    tiles = [(s, i, j) for s in range(NSEG) for i in reversed(range(NT)) for j in range(i + 1)]

    def attend(groups, true_max, side=()):
        blocks = [(k, *t) for k in range(len(groups)) for t in tiles]
        row = _iota((GP, T), 0)
        lane = _iota((GP, T), 1)
        mz_mask = jnp.zeros((GP, T), jnp.bool_)
        for h in range(HG):
            in_row = ((row >= h * DH) & (row < (h + 1) * DH)) | (row == GR + h)
            mz_mask = mz_mask | (in_row & (lane >= h * DH) & (lane < (h + 1) * DH))
        row8 = _iota((8, T), 0)
        st, col_max, acc, mz = {}, {}, {}, {}

        def scores(n):
            k, s, i, j = blocks[n]
            cols = pl.ds(i * T, T)

            def qk(lo, cnt, q, first):
                parts = [jnp.zeros((first // 2, T), U32), q,
                         jnp.zeros(((T - first) // 2 - q.shape[0], T), U32)]
                return _dot(_bf(kn_v[s, groups[k], pl.ds((j * T + lo) // 2, cnt // 2), :]),
                            _bf(jnp.concatenate([p for p in parts if p.shape[0]], axis=0)))

            def bias(r):
                return bias_v[pl.ds(T + r * QT, QT), :]

            for h in range(HG):
                q = qs_v[s, groups[k], h, :, cols]
                if true_max:
                    t = qk(0, T, q, 16 * h)
                    if j == i:
                        t = t + pltpu.roll(bias_v[pl.ds(0, T), :], h * QT, 1)
                    st[n, h] = t
                    m = jnp.max(t, axis=0, keepdims=True)
                    col_max[s, i, h] = jnp.maximum(col_max[s, i, h], m) if j else m
                elif j + 1 < i:
                    st[n, h] = qk(0, T, q, 16 * h)
                elif j < i:
                    t = qk(0, T + QT, q, 16 * h)
                    st[n, h], st[n + 1, h] = t[:T], t[T:] + bias(h)
                elif i == 0:
                    st[n, h] = qk(0, QT, q, 16 * h) + bias(h)
            if j == i and not true_max:
                for h in range(2):
                    t = qk(QT, 2 * QT, qx_v[s, groups[k], pl.ds(32 * h, 32), cols], 16 * h)
                    st[n, 'pair', h] = t[:QT], t[QT:] + bias(4 + h)
                for c in (1, 3):
                    st[n, 'quad', c] = bias(6) + qk(
                        c * QT, QT, qx_v[s, groups[k], pl.ds(44 + 20 * c, 40), cols], 0)

        def probs(n):
            k, s, i, j = blocks[n]
            if true_max:
                return [jnp.exp2(st.pop((n, h)) - col_max[s, i, h]) for h in range(HG)]
            if j < i:
                return [jnp.exp2(st.pop((n, h))) for h in range(HG)]
            slot = _iota((QT, T), 1) >> 5
            quad = {c: jnp.exp2(st.pop((n, 'quad', c))) for c in (1, 3)}
            pair = [[jnp.exp2(t) for t in st.pop((n, 'pair', h))] for h in range(2)]
            out = []
            for h in range(HG):
                late = ((slot - h) & 3) >= 2
                out.append(jnp.concatenate([
                    jnp.exp2(st.pop((n, h))),
                    jnp.where(late, pair[h % 2][0], jnp.where(slot == (1 + h) % HG, quad[1], 0.0)),
                    jnp.where(late, pair[h % 2][1], 0.0),
                    jnp.where(slot == (3 + h) % HG, quad[3], 0.0)], axis=0))
            return out

        def values(n):
            k, s, i, j = blocks[n]
            for h, p in enumerate(probs(n)):
                w = vt_v[s, groups[k], pl.ds(16 * h, 24), pl.ds(j * T, T)]
                if h < HG - 1:
                    w = jnp.concatenate([w[:16], jnp.where(row8 == 5 + h, 1.0, w[16:])], axis=0)
                else:
                    w = jnp.concatenate([jnp.where(row8 == 4, 1.0, w[:8]), w[8:]], axis=0)
                a = _dot(w, p.astype(BF16))
                acc[h] = a + acc[h] if j else a
                if j == i:
                    acc_v[s, groups[k], pl.ds(24 * h, 24), pl.ds(i * T, T)] = acc[h]

        def mem_update(k, s):
            pk = _phi(_bf(kn_v[s, groups[k]]).astype(F32)).astype(BF16)
            va = jnp.concatenate([vt_v[s, groups[k]], jnp.ones((GP - GR, L), F32)], axis=0)
            upd = jnp.where(mz_mask, _dot(va, pk), 0.0)
            mz[k] = mz[k] + upd if s else upd

        lag = NT + 1 if true_max else LAG
        for n in range(len(blocks) + lag):
            step = n % (len(tiles) // NSEG)
            if n < len(blocks):
                scores(n)
                k, s = blocks[n][:2]
                if s > 0 and step == MEM_READ_STEP and not true_max:
                    mem_v[s - 1, groups[k]] = _dot(mz[k][:, :GP], _bf(pq_v[s, groups[k]]))
                if s < NSEG - 1 and step == MEM_UPDATE_STEP and not true_max:
                    mem_update(k, s)
            if n >= lag:
                values(n - lag)
            if side and n >= FFN_FIRST_STEP and step in FFN_STEPS:
                side.pop(0)()
        assert not side

    def finish(g, s, i, seg):
        row8 = _iota((8, T), 0)
        cols = pl.ds(i * T, T)
        acc = [acc_v[seg, g, pl.ds(24 * h, 24), cols] for h in range(HG)]
        acc = [pltpu.roll(t, T - h * QT, 1) if h else t for h, t in enumerate(acc)]
        sums = jnp.where(row8 < 5, acc[3][:8], acc[2][16:])
        den = sums = jnp.where(row8 == 5, acc[0][16:], jnp.where(row8 == 6, acc[1][16:], sums))
        if s > 0:
            mem = mem_v[s - 1, g, :, cols]
            den = jnp.where(row8 < 4, mem[GR:] + 1e-6, sums)
        coef = gate_v[pl.ds(_aligned(g * 8, 8), 8), :] / den

        def spread(lo, mid, hi):
            out = [lo[0], mid[0]]
            for h in range(1, HG):
                out += [jnp.where(row8 < 2 * h, hi[h - 1], lo[h]), mid[h]]
            return jnp.concatenate(out + [hi[HG - 1]], axis=0)

        cl = [jnp.broadcast_to(coef[r:r + 1], (8, T)) for r in (5, 6, 7, 4)]
        o = spread(*[[t[r:r + 8] for t in acc] for r in (0, 8, 16)]) * spread(cl, cl, cl)
        if s > 0:
            cm = [jnp.broadcast_to(coef[r:r + 1], (8, T)) for r in range(HG)]
            o = o + mem[:GR] * spread(cm, cm, cm)
        ot_v[s, pl.ds(_aligned(g * GR, 8), GR), cols] = o
        return sums

    def output(finish_segment):
        pieces = [(s, 0, D) for s in range(NSEG - 1)]
        pieces += [(NSEG - 1, r, n) for r, n in ((0, 288), (288, 192), (480, 96))]
        out_cp = []
        finish_segment(0)
        for i, (s, r, n) in enumerate(pieces):
            rows = pl.ds(r, n)
            if s + 1 < NSEG:
                finish_segment(s + 1)
            att = _dot(_bf(wt_v[pl.ds(WO + r // 2, n // 2), :]), ot_v[s].astype(BF16))
            if s + 2 < NSEG:
                acc_v[0, 0, :8, :T] = att[-8:, :T]
            out_v[s, rows, :] = (x_v[s, rows, :].astype(F32) + att
                                 + _bf(xn_v[s, pl.ds(r // 2, n // 2), :]).astype(F32)).astype(BF16)
            out_cp.append(pltpu.make_async_copy(
                out_v.at[s, rows, :], out_hbm.at[rows, pl.ds(s * L, L)], out_sem.at[i]))
            out_cp[-1].start()
        return out_cp

    bias_v[pl.ds(0, T), :] = jnp.where(_iota((T, T), 0) <= _iota((T, T), 1), 0.0, NEG)
    for i, (rot, width) in enumerate([(h, T) for h in range(HG)] + [(0, 2 * QT), (1, 2 * QT), (0, QT)]):
        bias_v[pl.ds(T + i * QT, QT), :] = jnp.where(
            _iota((QT, T), 0) <= ((_iota((QT, T), 1) - rot * QT) & (width - 1)), 0.0, NEG)
    wo_v[pl.ds(D, DP - D), :] = jnp.zeros((DP - D, D), BF16)
    for s in range(NSEG):
        ot_v[s, pl.ds(D + 8, DP - D - 8), :] = jnp.zeros((DP - D - 8, L), F32)

    x_cp[0].wait()
    for t in range(NT):
        layernorm(0, t)
    wv_cp.wait()
    transpose_weight(2)
    run(project(project_v, 0, range(3)))
    for c in [*small_cp, wq_cp]:
        c.wait()
    small_tables()
    project_v(0, 3)
    transpose_weight(0)
    run(project(project_q, 0, range(3)))
    for c in [wk_cp, x_cp[1]]:
        c.wait()
    project_q(0, 3)
    transpose_weight(1)
    run(project(project_k, 0, range(3)), norm=1)
    run(project(project_k, 0, [3]) + project(project_k, 1) + project(project_v, 1, [0]))
    for c in [*x_cp[2:], wo_cp]:
        c.wait()
    run(project(project_v, 1, range(1, 4)) + project(project_q, 1, range(3)), norm=2)
    project_q(1, 3)
    for c in range(0, DP - T, T):
        transpose_wo(c)
    run(project(project_v, 2) + project(project_k, 2), norm=3)
    run(project(project_q, 2) + project(project_v, 3, [3]))
    tokens = top2()
    run(project(project_k, 3) + project(project_q, 3))
    for p in range(3):
        if p < 2:
            gather(tokens, p * L)
        project_v(3, p)

    attend(list(range(NG)), False,
           [ffn_wait] + [f for c in range(0, FF, L) for f in ffn_steps(c)] + [ffn_done])

    lim = []

    def finish_and_watch(s):
        for g in range(NG):
            for i in range(NT):
                sums = finish(g, s, i, s + zero if s else s)
                lim[:] = [jnp.minimum(lim[0], sums), jnp.maximum(lim[1], sums)] if lim else [sums, sums]

    out_cp = output(finish_and_watch)
    safe = (_iota((8, T), 0) < 4) | ((lim[0] >= SAFE_LO) & (lim[1] <= SAFE_HI))
    unsafe = jnp.min(jnp.where(safe, 1, 0)) == 0
    for c in out_cp:
        c.wait()

    @pl.when(unsafe)
    def _():
        def redo(g, carry):
            attend([g], True)
            for s in range(NSEG):
                for i in range(NT):
                    finish(g, s, i, s)
            return carry

        jax.lax.fori_loop(0, NG, redo, 0)
        for c in output(lambda s: None):
            c.wait()


@jax.jit
def pallas_parallel_sum__memory_aug_infini_attn__moe_arch_mod__prompt_kernel(
    A_x: jax.Array,
    A_wq: jax.Array,
    A_wk: jax.Array,
    A_wv: jax.Array,
    A_wo: jax.Array,
    A_beta: jax.Array,
    B_x: jax.Array,
    B_w_r: jax.Array,
    B_w_gate: jax.Array,
    B_w_up: jax.Array,
    B_w_down: jax.Array,
):
    del B_x
    assert A_x.shape == (1, S, D) and B_w_gate.shape == (D, FF)
    hbm = pl.BlockSpec(memory_space=pl.ANY)
    out_t = pl.pallas_call(
        _kernel,
        out_shape=jax.ShapeDtypeStruct((D, S), BF16),
        in_specs=[hbm] * 10,
        out_specs=hbm,
        scratch_shapes=[
            pltpu.VMEM((D,), BF16),
            pltpu.VMEM((H,), BF16),
            pltpu.VMEM((NSEG, D, L), BF16),
            pltpu.VMEM((3, D, D), BF16),
            pltpu.VMEM((DP, D), BF16),
            pltpu.VMEM((WO + D // 2, DP), U32),
            pltpu.VMEM((NSEG, D // 2, L), U32),
            pltpu.VMEM((NSEG, NG, HG, 16, L), U32),
            pltpu.VMEM((NSEG, NG, 144, L), U32),
            pltpu.VMEM((NSEG, NG, GP // 2, L), U32),
            pltpu.VMEM((NSEG, NG, L // 2, T), U32),
            pltpu.VMEM((NSEG, NG, GR, L), F32),
            pltpu.VMEM((NSEG, NG, HG * 24, L), F32),
            pltpu.VMEM((NSEG - 1, NG, GP, L), F32),
            pltpu.VMEM((NSEG, DP, L), F32),
            pltpu.VMEM((NSEG, 8, L), F32),
            pltpu.VMEM((NG * 8, T), F32),
            pltpu.VMEM((T + 7 * QT, T), F32),
            pltpu.VMEM((8, D), F32),
            pltpu.VMEM((8, D), F32),
            pltpu.VMEM((8, T), F32),
            pltpu.VMEM((D, FF), BF16),
            pltpu.VMEM((D, FF), BF16),
            pltpu.VMEM((D, FF), BF16),
            pltpu.VMEM((NSEG, D, L), BF16),
            pltpu.SemaphoreType.DMA((NSEG + 9,)),
            pltpu.SemaphoreType.DMA((NSEG + 2,)),
        ],
        compiler_params=pltpu.CompilerParams(vmem_limit_bytes=100 * 2 ** 20),
        name="infini_mod",
    )(B_w_r, A_beta, A_x[0].T, A_wq, A_wk, A_wv, A_wo, B_w_gate, B_w_up, B_w_down.T)
    return out_t.T[None]
```

```python
import math
from functools import partial

import jax
import jax.numpy as jnp
import jax.experimental.pallas as pl
import jax.experimental.pallas.tpu as pltpu

D = 576
S = 2048
H = 32
DH = D // H
NSEG = 4
L = S // NSEG
FF = 4608
HG = 4
NG = H // HG
GR = HG * DH
GP = 80
T = 128
QT = T // HG
NT = L // T
CH = 2 * GR
NCH = D // CH
DP = 640
WO = 3 * D // 2 + 8

F32 = jnp.float32
BF16 = jnp.bfloat16
U32 = jnp.uint32
QSCALE = (DH ** -0.5) * math.log2(math.e)
NEG = -1e30
SAFE_LO, SAFE_HI = 2.0 ** -30, 2.0 ** 30
LAG = 3
FIN = 1
LNPIN = 1
HEAD = 384
NV = 1
FFN_FIRST_STEP = 30
FFN_STEPS = (0, 1, 2, 4, 5)


def _iota(shape, dim):
    return jax.lax.broadcasted_iota(jnp.int32, shape, dim)


def _round_bf16(t):
    return t.astype(BF16).astype(F32)


def _pack(t):
    return pltpu.bitcast(t.astype(BF16), U32)


def _bf(t):
    return pltpu.bitcast(t, BF16)


def _phi(t):
    return jnp.where(t > 0, t + 1.0, jnp.exp(t))


def _dot(a, b):
    return jax.lax.dot_general(a, b, (((1,), (0,)), ((), ())), preferred_element_type=F32)


def _dot_nt(a, b):
    return jax.lax.dot_general(a, b, (((1,), (1,)), ((), ())), preferred_element_type=F32)


def _aligned(i, n):
    return i if isinstance(i, int) else pl.multiple_of(i, n)


def _kernel(wr_hbm, beta_hbm, x_hbm, wq_hbm, wk_hbm, wv_hbm, wo_hbm, wg_hbm, wu_hbm, wd_hbm,
            out_hbm,
            wr_v, beta_v, x_v, wraw_v, wo_v, wt_v, xn_v, qs_v, qx_v, pq_v, kn_v, vt_v, acc_v,
            mz_v, mem_v, ot_v, r_v, gate_v, bias_v, xs_v, y_v, rs_v, wg_v, wu_v, wd_v, out_v,
            in_sem, out_sem):
    x_cp = [pltpu.make_async_copy(x_hbm.at[:, pl.ds(s * L, L)], x_v.at[s], in_sem.at[s])
            for s in range(NSEG)]
    head, rest = pl.ds(0, HEAD), pl.ds(HEAD, D - HEAD)
    wq_cp, wk_cp, wv_cp, wv_rest_cp, wo_cp, *more_cp = [
        pltpu.make_async_copy(src, dst, in_sem.at[NSEG + i]) for i, (src, dst) in enumerate((
            (wq_hbm, wraw_v.at[0]), (wk_hbm, wraw_v.at[1]),
            (wv_hbm.at[:, head], wraw_v.at[2, :, head]), (wv_hbm.at[:, rest], wraw_v.at[2, :, rest]),
            (wo_hbm, wo_v.at[pl.ds(0, D)]), (wr_hbm, wr_v), (beta_hbm, beta_v),
            (wg_hbm, wg_v), (wu_hbm, wu_v), (wd_hbm, wd_v)))]
    small_cp, ffn_cp = more_cp[:2], more_cp[2:]
    for c in [x_cp[0], wv_cp, wv_rest_cp, *small_cp, wq_cp, wk_cp, *x_cp[1:], wo_cp, *ffn_cp]:
        c.start()

    zero = jnp.min(_iota((8, T), 1))
    zeros = _iota((8, T), 1) * zero
    marks = []

    def marker(*values):
        out = pltpu.bitcast(values[0], jnp.int32)
        for t in values[1:]:
            out = out | pltpu.bitcast(t, jnp.int32)
        return out & zeros

    def tied(t, mark):
        head = pltpu.bitcast(pltpu.bitcast(t[:8, :T], jnp.int32) | mark, t.dtype)
        return jnp.concatenate([jnp.concatenate([head, t[:8, T:]], axis=1), t[8:]], axis=0)

    def layernorm(s, t):
        cols = pl.ds(t * T, T)
        shift = jnp.broadcast_to(x_v[s, pl.ds(0, 16), cols].astype(F32)[:1], (16, T))
        for d in range(0, D, 16):
            xc = x_v[s, pl.ds(d, 16), cols].astype(F32) - shift
            s1, s2 = (s1 + xc, s2 + xc * xc) if d else (xc, xc * xc)
        m = jnp.sum(s1, axis=0, keepdims=True) * (1.0 / D)
        v = jnp.maximum(jnp.sum(s2, axis=0, keepdims=True) * (1.0 / D) - m * m, 0.0)
        m = jnp.broadcast_to(_round_bf16(m + shift[:1]), (16, T))
        inv = jnp.broadcast_to(
            1.0 / _round_bf16(jnp.sqrt(_round_bf16(_round_bf16(v) + 1e-5))), (16, T))
        for d in range(0, D, 16):
            x = x_v[s + zero, pl.ds(d, 16), cols].astype(F32)
            xn_v[s, pl.ds(d, 16), cols] = (_round_bf16(x - m) * inv).astype(BF16)
        return marker(xn_v[s + zero, :16, cols])

    def transpose_weight(i, lo=0, hi=D):
        for c in range(lo, hi, T):
            n = min(T, D - c)
            wt_v[pl.ds((i * D + c) // 2, n // 2), pl.ds(0, D)] = pltpu.bitcast(
                wraw_v[i, :, pl.ds(c, n)].T, U32)

    def transpose_wo(c):
        wt_v[pl.ds(WO, D // 2), pl.ds(c, T)] = pltpu.bitcast(wo_v[pl.ds(c, T), :].T, U32)

    def proj(s, row, n, keep=None):
        w = wt_v[pl.ds(row if not isinstance(row, int) else row // 2, n // 2), pl.ds(0, D)]
        mark = marks.pop(0) if len(marks) > 1 else None
        w = _bf(w if mark is None else tied(w, mark))
        return _dot(w.astype(F32)[:keep] if keep else w, xn_v[s])

    def project_q(s, p):
        zpad = jnp.zeros((GP - GR, L), F32)
        row32 = _iota((32, L), 0)
        slot = _iota((16, T), 1) >> 5
        q = proj(s, p * CH, CH)
        for j in range(2):
            g = 2 * p + j
            qg = q[j * GR:(j + 1) * GR]
            if s:
                pq_v[s, g] = _pack(jnp.concatenate([_phi(qg), zpad], axis=0))
            qg = jnp.concatenate([qg * QSCALE, zpad], axis=0)
            qh = [_pack(jnp.where((row32 >= 2 * h) & (row32 < 2 * h + DH), qg[16 * h:16 * h + 32], 0.0))
                  for h in range(HG)]
            for t in range(0, L, T):
                cols = pl.ds(t, T)
                rot = [pltpu.roll(w[:, t:t + T], h * QT, 1) if h else w[:, t:t + T]
                       for h, w in enumerate(qh)]
                for h in range(HG):
                    qs_v[s, g, h, :, cols] = rot[h]
                    qx_v[s, g, pl.ds(16 * (h // 2 + h % 2 * 2), 16), cols] = jnp.where(
                        ((slot - h) & 3) >= 2, rot[h], 0)
                for c in (1, 3):
                    ws = [jnp.where(slot == (c + h) % HG, rot[h], 0) for h in range(HG)]
                    qx_v[s, g, pl.ds(44 + 20 * c, 40), cols] = jnp.concatenate(
                        [ws[0][:8], *[a[8:] | b[:8] for a, b in zip(ws, ws[1:])], ws[-1][8:]], axis=0)
        marks.append(marker(qs_v[s + zero, g, 0, :8, :T], qx_v[s + zero, g, :8, :T],
                            *([pq_v[s + zero, g, :8, :T]] if s else [])))

    def project_k(s, p):
        k = proj(s, D + p * CH, CH)
        for j in range(2):
            kg = jnp.concatenate([k[j * GR:(j + 1) * GR], jnp.zeros((T - GR, L), F32)], axis=0)
            kn_v[s, 2 * p + j] = pltpu.bitcast(kg.astype(BF16).T, U32)
        marks.append(marker(kn_v[s + zero, 2 * p, :8, :]))

    def project_v(s, p):
        extra = 16 if p == NCH - 1 else 0
        row = 2 * D + p * CH
        if extra and s == NSEG - 1:
            row = pl.multiple_of(row // 2 + 8 * zero, 8)
        v = proj(s, row, CH + extra, CH + 8 if extra else None)
        for j in range(2):
            vt_v[s, 2 * p + j] = v[j * GR:(j + 1) * GR]
        if extra:
            r_v[s] = v[CH:CH + 8]
        marks.append(None)

    def mem_update(s, g):
        row, lane = _iota((GP, T), 0), _iota((GP, T), 1)
        keep = None
        for h in range(HG):
            rows = ((row >= h * DH) & (row < (h + 1) * DH)) | (row == GR + h)
            block = rows & (lane >= h * DH) & (lane < (h + 1) * DH)
            keep = keep | block if h else block
        pk = _phi(_bf(kn_v[s, g]).astype(F32))
        z = jnp.broadcast_to(jnp.sum(pk, axis=0, keepdims=True), (GP - GR, T))
        upd = jnp.where(keep, jnp.concatenate([_dot(vt_v[s, g], pk.astype(BF16)), z], axis=0), 0.0)
        mz_v[s, g] = mz_v[s - 1, g] + upd if s else upd

    def mem_read(s, g):
        mem_v[s - 1, g] = _dot(mz_v[s - 1, g, :, pl.ds(0, GP)], _bf(pq_v[s, g]))

    def project(f, s, ps=range(NCH), then=()):
        def step(p):
            f(s, p)
            for g in (2 * p, 2 * p + 1):
                for fn, seg in then:
                    fn(seg, g)

        return [partial(step, p) for p in ps]

    def run(dots, norm=None):
        for i, f in enumerate(dots):
            f()
            for t in range(i * NT // len(dots), (i + 1) * NT // len(dots)) if norm else ():
                mark = layernorm(norm, t)
                if LNPIN:
                    marks[-1] = mark if marks[-1] is None else marks[-1] | mark

    def small_tables():
        wt_v[pl.ds(3 * D // 2, 8), pl.ds(0, D)] = _pack(
            jnp.broadcast_to(wr_v[...].astype(F32).reshape(1, D), (16, D)))
        sg = jax.nn.sigmoid(beta_v[...].astype(F32).reshape(1, H))
        row = _iota((NG * 8, H), 0)
        head = (row >> 3) * HG + ((row + jnp.where((row & 4) != 0, 3, 0)) & 3)
        gate = jnp.sum(jnp.where(_iota((NG * 8, H), 1) == head,
                                 jnp.broadcast_to(sg, (NG * 8, H)), 0.0), axis=1, keepdims=True)
        gate = jnp.where((_iota((NG * 8, 1), 0) & 4) != 0, 1.0 - gate, gate)
        gate_v[...] = jnp.broadcast_to(gate, (NG * 8, T))

    def top2():
        r = _round_bf16(jnp.concatenate([r_v[s] for s in range(NSEG)], axis=1))
        pos = _iota((8, S), 1)
        m1 = jnp.max(r, axis=1, keepdims=True)
        i1 = jnp.min(jnp.where(r == m1, pos, S), axis=1, keepdims=True)
        r2 = jnp.where(pos == i1, -jnp.inf, r)
        m2 = jnp.max(r2, axis=1, keepdims=True)
        i2 = jnp.min(jnp.where((r2 == m2) & (pos != i1), pos, S), axis=1, keepdims=True)
        sub = _iota((8, S), 0)
        onehot = jnp.where(((sub == 0) & (pos == i1)) | ((sub == 1) & (pos == i2)), 1.0, 0.0)
        for s in range(NSEG):
            ot_v[s, pl.ds(D, 8), :] = onehot[:, s * L:(s + 1) * L]
        rs_v[...] = jnp.broadcast_to(
            jax.nn.sigmoid(jnp.where(_iota((8, 1), 0) == 0, m1, m2)), (8, T))
        return [jnp.clip(jnp.min(i), 0, S - 1) for i in (i1, i2)]

    def gather(tokens, d):
        n = min(L, D - d)
        for c, tok in enumerate(tokens):
            tile = xn_v[tok >> 9, pl.ds(d, n), pl.ds(pl.multiple_of(tok & (L - T), T), T)]
            pick = (_iota((8, T), 0) == c) & (_iota((8, T), 1) == (tok & (T - 1)))
            row = _dot_nt(jnp.where(pick, 1.0, 0.0), tile)
            rows = row + rows if c else row
        xs_v[:, pl.ds(d, n)] = rows
        y_v[:, pl.ds(d, n)] = jnp.zeros((8, n), F32)

    def ffn_steps(c):
        cols = pl.ds(c, L)
        acc = {}

        def gate_up(m, d):
            rows = pl.ds(d, min(T, D - d))
            a = _dot(xs_v[:, rows], (wg_v, wu_v)[m][rows, cols])
            acc[m] = a + acc[m] if d else a

        def down(d):
            rows = pl.ds(d, min(T, D - d))
            if d == 0:
                acc[2] = acc[0] * jax.nn.sigmoid(acc[0]) * acc[1]
            y_v[:, rows] += _dot_nt(acc[2], wd_v[rows, cols])

        return ([partial(gate_up, m, d) for m in range(2) for d in range(0, D, T)]
                + [partial(down, d) for d in range(0, D, T)])

    def ffn_wait():
        for c in ffn_cp:
            c.wait()

    def ffn_done():
        y = y_v[...] * rs_v[:, pl.ds(0, 1)]
        wo_v[pl.ds(D, 16), :] = jnp.concatenate([y, jnp.zeros((8, D), F32)], axis=0).astype(BF16)
        transpose_wo(DP - T)

    tiles = [(s, i, j) for s in range(NSEG) for i in reversed(range(NT)) for j in range(i + 1)]

    def attend(groups, true_max, side=()):
        blocks = [(k, *t) for k in range(len(groups)) for t in tiles]
        row8 = _iota((8, T), 0)
        st, col_max, acc = {}, {}, {}

        def scores(n):
            k, s, i, j = blocks[n]
            cols = pl.ds(i * T, T)

            def qk(lo, cnt, q, first):
                parts = [jnp.zeros((first // 2, T), U32), q,
                         jnp.zeros(((T - first) // 2 - q.shape[0], T), U32)]
                return _dot(_bf(kn_v[s, groups[k], pl.ds((j * T + lo) // 2, cnt // 2), :]),
                            _bf(jnp.concatenate([p for p in parts if p.shape[0]], axis=0)))

            def bias(r):
                return bias_v[pl.ds(T + r * QT, QT), :]

            for h in range(HG):
                q = qs_v[s, groups[k], h, :, cols]
                if true_max:
                    t = qk(0, T, q, 16 * h)
                    if j == i:
                        t = t + pltpu.roll(bias_v[pl.ds(0, T), :], h * QT, 1)
                    st[n, h] = t
                    m = jnp.max(t, axis=0, keepdims=True)
                    col_max[s, i, h] = jnp.maximum(col_max[s, i, h], m) if j else m
                elif j + 1 < i:
                    st[n, h] = qk(0, T, q, 16 * h)
                elif j < i:
                    t = qk(0, T + QT, q, 16 * h)
                    st[n, h], st[n + 1, h] = t[:T], t[T:] + bias(h)
                elif i == 0:
                    st[n, h] = qk(0, QT, q, 16 * h) + bias(h)
            if j == i and not true_max:
                for h in range(2):
                    t = qk(QT, 2 * QT, qx_v[s, groups[k], pl.ds(32 * h, 32), cols], 16 * h)
                    st[n, 'pair', h] = t[:QT], t[QT:] + bias(4 + h)
                for c in (1, 3):
                    st[n, 'quad', c] = bias(6) + qk(
                        c * QT, QT, qx_v[s, groups[k], pl.ds(44 + 20 * c, 40), cols], 0)

        def probs(n):
            k, s, i, j = blocks[n]
            if true_max:
                return [jnp.exp2(st.pop((n, h)) - col_max[s, i, h]) for h in range(HG)]
            if j < i:
                return [jnp.exp2(st.pop((n, h))) for h in range(HG)]
            slot = _iota((QT, T), 1) >> 5
            quad = {c: jnp.exp2(st.pop((n, 'quad', c))) for c in (1, 3)}
            pair = [[jnp.exp2(t) for t in st.pop((n, 'pair', h))] for h in range(2)]
            out = []
            for h in range(HG):
                late = ((slot - h) & 3) >= 2
                out.append(jnp.concatenate([
                    jnp.exp2(st.pop((n, h))),
                    jnp.where(late, pair[h % 2][0], jnp.where(slot == (1 + h) % HG, quad[1], 0.0)),
                    jnp.where(late, pair[h % 2][1], 0.0),
                    jnp.where(slot == (3 + h) % HG, quad[3], 0.0)], axis=0))
            return out

        def values(n):
            k, s, i, j = blocks[n]
            for h, p in enumerate(probs(n)):
                w = vt_v[s, groups[k], pl.ds(16 * h, 24), pl.ds(j * T, T)]
                if h < HG - 1:
                    w = jnp.concatenate([w[:16], jnp.where(row8 == 5 + h, 1.0, w[16:])], axis=0)
                else:
                    w = jnp.concatenate([jnp.where(row8 == 4, 1.0, w[:8]), w[8:]], axis=0)
                a = _dot(w, p.astype(BF16))
                acc[h] = a + acc[h] if j else a
                if j == i:
                    acc_v[s, groups[k], pl.ds(24 * h, 24), pl.ds(i * T, T)] = acc[h]

        lag = NT + 1 if true_max else LAG
        for n in range(len(blocks)):
            step = n % (len(tiles) // NSEG)
            scores(n)
            if n >= lag:
                values(n - lag)
            if side and n >= FFN_FIRST_STEP and step in FFN_STEPS:
                side.pop(0)()
        assert not side
        return [partial(values, n) for n in range(len(blocks) - lag, len(blocks))]

    def finish(g, s, i, seg):
        row8 = _iota((8, T), 0)
        cols = pl.ds(i * T, T)
        acc = [acc_v[seg, g, pl.ds(24 * h, 24), cols] for h in range(HG)]
        acc = [pltpu.roll(t, T - h * QT, 1) if h else t for h, t in enumerate(acc)]
        sums = jnp.where(row8 < 5, acc[3][:8], acc[2][16:])
        den = sums = jnp.where(row8 == 5, acc[0][16:], jnp.where(row8 == 6, acc[1][16:], sums))
        if s > 0:
            mem = mem_v[s - 1, g, :, cols]
            den = jnp.where(row8 < 4, mem[GR:] + 1e-6, sums)
        coef = gate_v[pl.ds(_aligned(g * 8, 8), 8), :] / den

        def spread(lo, mid, hi):
            out = [lo[0], mid[0]]
            for h in range(1, HG):
                out += [jnp.where(row8 < 2 * h, hi[h - 1], lo[h]), mid[h]]
            return jnp.concatenate(out + [hi[HG - 1]], axis=0)

        cl = [jnp.broadcast_to(coef[r:r + 1], (8, T)) for r in (5, 6, 7, 4)]
        o = spread(*[[t[r:r + 8] for t in acc] for r in (0, 8, 16)]) * spread(cl, cl, cl)
        if s > 0:
            cm = [jnp.broadcast_to(coef[r:r + 1], (8, T)) for r in range(HG)]
            o = o + mem[:GR] * spread(cm, cm, cm)
        ot_v[s, pl.ds(_aligned(g * GR, 8), GR), cols] = o
        return sums

    def output(finish_segment, tail=()):
        pieces = [(s, 0, D) for s in range(NSEG - 1)]
        pieces += [(NSEG - 1, r, n) for r, n in ((0, 288), (288, 192), (480, 96))]
        out_cp = []
        finish_segment(0)
        for i, (s, r, n) in enumerate(pieces):
            rows = pl.ds(r, n)
            if s + 1 < NSEG:
                finish_segment(s + 1)
            att = _dot(_bf(wt_v[pl.ds(WO + r // 2, n // 2), :]), ot_v[s].astype(BF16))
            for f in tail if i == 0 else ():
                f()
            if s + 2 < NSEG:
                acc_v[0, 0, :8, :T] = att[-8:, :T]
            out_v[s, rows, :] = (x_v[s, rows, :].astype(F32) + att
                                 + xn_v[s, rows, :].astype(F32)).astype(BF16)
            out_cp.append(pltpu.make_async_copy(
                out_v.at[s, rows, :], out_hbm.at[rows, pl.ds(s * L, L)], out_sem.at[i]))
            out_cp[-1].start()
        return out_cp

    bias_v[pl.ds(0, T), :] = jnp.where(_iota((T, T), 0) <= _iota((T, T), 1), 0.0, NEG)
    for i, (rot, width) in enumerate([(h, T) for h in range(HG)] + [(0, 2 * QT), (1, 2 * QT), (0, QT)]):
        bias_v[pl.ds(T + i * QT, QT), :] = jnp.where(
            _iota((QT, T), 0) <= ((_iota((QT, T), 1) - rot * QT) & (width - 1)), 0.0, NEG)
    wo_v[pl.ds(D, DP - D), :] = jnp.zeros((DP - D, D), BF16)
    for s in range(NSEG):
        ot_v[s, pl.ds(D + 8, DP - D - 8), :] = jnp.zeros((DP - D - 8, L), F32)

    x_cp[0].wait()
    for t in range(NT):
        layernorm(0, t)
    wv_cp.wait()
    transpose_weight(2, 0, HEAD)
    run(project(project_v, 0, range(NV)))
    wv_rest_cp.wait()
    transpose_weight(2, HEAD)
    run(project(project_v, 0, range(NV, 3)))
    for c in [*small_cp, wq_cp]:
        c.wait()
    small_tables()
    project_v(0, 3)
    transpose_weight(0)
    run(project(project_q, 0, range(3)))
    for c in [wk_cp, x_cp[1]]:
        c.wait()
    project_q(0, 3)
    transpose_weight(1)
    run(project(project_k, 0, range(3)), norm=1)
    run(project(project_k, 0, [3]) + project(project_k, 1, then=[(mem_update, 0)])
        + project(project_v, 1, [0]))
    for c in [*x_cp[2:], wo_cp]:
        c.wait()
    run(project(project_v, 1, range(1, 4)) + project(project_q, 1, range(3)), norm=2)
    project_q(1, 3)
    for c in range(0, DP - T, T):
        transpose_wo(c)
    run(project(project_v, 2) + project(project_k, 2), norm=3)
    run(project(project_q, 2) + project(project_v, 3, [3]))
    tokens = top2()
    run(project(project_k, 3, then=[(mem_update, 1)]) + project(project_q, 3, then=[(mem_read, 1)])
        + project(project_v, 3, [0, 1], then=[(mem_update, 2), (mem_read, 2)]))
    project_v(3, 2)
    for g in range(NG // 2, NG):
        mem_update(2, g)
        mem_read(2, g)
    for g in range(NG):
        mem_read(3, g)
    for d in range(0, D, L):
        gather(tokens, d)

    tail = attend(list(range(NG)), False,
                  [ffn_wait] + [f for c in range(0, FF, L) for f in ffn_steps(c)] + [ffn_done])

    lim = []

    def finish_and_watch(s):
        for g in range(NG):
            for i in range(NT):
                sums = finish(g, s, i, s + zero if s >= FIN else s)
                lim[:] = [jnp.minimum(lim[0], sums), jnp.maximum(lim[1], sums)] if lim else [sums, sums]

    out_cp = output(finish_and_watch, tail)
    safe = (_iota((8, T), 0) < 4) | ((lim[0] >= SAFE_LO) & (lim[1] <= SAFE_HI))
    unsafe = jnp.min(jnp.where(safe, 1, 0)) == 0
    for c in out_cp:
        c.wait()

    @pl.when(unsafe)
    def _():
        def redo(g, carry):
            for f in attend([g], True):
                f()
            for s in range(NSEG):
                for i in range(NT):
                    finish(g, s, i, s)
            return carry

        jax.lax.fori_loop(0, NG, redo, 0)
        for c in output(lambda s: None):
            c.wait()


@jax.jit
def pallas_parallel_sum__memory_aug_infini_attn__moe_arch_mod__prompt_kernel(
    A_x: jax.Array,
    A_wq: jax.Array,
    A_wk: jax.Array,
    A_wv: jax.Array,
    A_wo: jax.Array,
    A_beta: jax.Array,
    B_x: jax.Array,
    B_w_r: jax.Array,
    B_w_gate: jax.Array,
    B_w_up: jax.Array,
    B_w_down: jax.Array,
):
    del B_x
    assert A_x.shape == (1, S, D) and B_w_gate.shape == (D, FF)
    hbm = pl.BlockSpec(memory_space=pl.ANY)
    out_t = pl.pallas_call(
        _kernel,
        out_shape=jax.ShapeDtypeStruct((D, S), BF16),
        in_specs=[hbm] * 10,
        out_specs=hbm,
        scratch_shapes=[
            pltpu.VMEM((D,), BF16),
            pltpu.VMEM((H,), BF16),
            pltpu.VMEM((NSEG, D, L), BF16),
            pltpu.VMEM((3, D, D), BF16),
            pltpu.VMEM((DP, D), BF16),
            pltpu.VMEM((WO + D // 2, DP), U32),
            pltpu.VMEM((NSEG, D, L), BF16),
            pltpu.VMEM((NSEG, NG, HG, 16, L), U32),
            pltpu.VMEM((NSEG, NG, 144, L), U32),
            pltpu.VMEM((NSEG, NG, GP // 2, L), U32),
            pltpu.VMEM((NSEG, NG, L // 2, T), U32),
            pltpu.VMEM((NSEG, NG, GR, L), F32),
            pltpu.VMEM((NSEG, NG, HG * 24, L), F32),
            pltpu.VMEM((NSEG - 1, NG, GP, T), F32),
            pltpu.VMEM((NSEG - 1, NG, GP, L), F32),
            pltpu.VMEM((NSEG, DP, L), F32),
            pltpu.VMEM((NSEG, 8, L), F32),
            pltpu.VMEM((NG * 8, T), F32),
            pltpu.VMEM((T + 7 * QT, T), F32),
            pltpu.VMEM((8, D), F32),
            pltpu.VMEM((8, D), F32),
            pltpu.VMEM((8, T), F32),
            pltpu.VMEM((D, FF), BF16),
            pltpu.VMEM((D, FF), BF16),
            pltpu.VMEM((D, FF), BF16),
            pltpu.VMEM((NSEG, D, L), BF16),
            pltpu.SemaphoreType.DMA((NSEG + 10,)),
            pltpu.SemaphoreType.DMA((NSEG + 2,)),
        ],
        compiler_params=pltpu.CompilerParams(vmem_limit_bytes=100 * 2 ** 20),
        name="infini_mod",
    )(B_w_r, A_beta, A_x[0].T, A_wq, A_wk, A_wv, A_wo, B_w_gate, B_w_up, B_w_down.T)
    return out_t.T[None]
```

```python
import math
from functools import partial

import jax
import jax.numpy as jnp
import jax.experimental.pallas as pl
import jax.experimental.pallas.tpu as pltpu

D = 576
S = 2048
H = 32
DH = D // H
NSEG = 4
L = S // NSEG
FF = 4608
HG = 4
NG = H // HG
GR = HG * DH
GP = 80
T = 128
QT = T // HG
NT = L // T
CH = 2 * GR
NCH = D // CH
DP = 640
HEAD = 3 * T
WO = 3 * D // 2 + 8

F32 = jnp.float32
BF16 = jnp.bfloat16
U32 = jnp.uint32
QSCALE = (DH ** -0.5) * math.log2(math.e)
NEG = -1e30
SAFE_LO, SAFE_HI = 2.0 ** -30, 2.0 ** 30
LAG = 2
FFN_FIRST_STEP = 30
FFN_STEPS = (0, 1, 2, 4, 5, 7)


def _iota(shape, dim):
    return jax.lax.broadcasted_iota(jnp.int32, shape, dim)


def _round_bf16(t):
    return t.astype(BF16).astype(F32)


def _pack(t):
    return pltpu.bitcast(t.astype(BF16), U32)


def _bf(t):
    return pltpu.bitcast(t, BF16)


def _phi(t):
    return jnp.where(t > 0, t + 1.0, jnp.exp(t))


def _dot(a, b):
    return jax.lax.dot_general(a, b, (((1,), (0,)), ((), ())), preferred_element_type=F32)


def _dot_nt(a, b):
    return jax.lax.dot_general(a, b, (((1,), (1,)), ((), ())), preferred_element_type=F32)


def _aligned(i, n):
    return i if isinstance(i, int) else pl.multiple_of(i, n)


def _kernel(wr_hbm, beta_hbm, x_hbm, wq_hbm, wk_hbm, wv_hbm, wo_hbm, wg_hbm, wu_hbm, wd_hbm,
            out_hbm,
            wr_v, beta_v, x_v, wraw_v, wo_v, wt_v, xn_v, qs_v, qx_v, pq_v, kn_v, vt_v, acc_v,
            mz_v, mem_v, ot_v, r_v, gate_v, bias_v, xs_v, y_v, rs_v, wg_v, wu_v, wd_v, out_v,
            in_sem, out_sem):
    x_cp = [pltpu.make_async_copy(x_hbm.at[:, pl.ds(s * L, L)], x_v.at[s], in_sem.at[s])
            for s in range(NSEG)]
    head, rest = pl.ds(0, HEAD), pl.ds(HEAD, D - HEAD)
    wq_cp, wk_cp, wv_cp, wv_rest_cp, wo_cp, *more_cp = [
        pltpu.make_async_copy(src, dst, in_sem.at[NSEG + i]) for i, (src, dst) in enumerate((
            (wq_hbm, wraw_v.at[0]), (wk_hbm, wraw_v.at[1]),
            (wv_hbm.at[:, head], wraw_v.at[2, :, head]), (wv_hbm.at[:, rest], wraw_v.at[2, :, rest]),
            (wo_hbm, wo_v.at[pl.ds(0, D)]), (wr_hbm, wr_v), (beta_hbm, beta_v),
            (wg_hbm, wg_v), (wu_hbm, wu_v), (wd_hbm, wd_v)))]
    small_cp, ffn_cp = more_cp[:2], more_cp[2:]
    for c in [x_cp[0], wv_cp, wv_rest_cp, *small_cp, wq_cp, wk_cp, *x_cp[1:], wo_cp, *ffn_cp]:
        c.start()

    zero = jnp.min(_iota((8, T), 1))
    zeros = _iota((8, T), 1) * zero
    marks = []

    def marker(*values):
        out = pltpu.bitcast(values[0], jnp.int32)
        for t in values[1:]:
            out = out | pltpu.bitcast(t, jnp.int32)
        return out & zeros

    def tied(t, mark):
        head = pltpu.bitcast(pltpu.bitcast(t[:8, :T], jnp.int32) | mark, t.dtype)
        return jnp.concatenate([jnp.concatenate([head, t[:8, T:]], axis=1), t[8:]], axis=0)

    def layernorm(s, t):
        cols = pl.ds(t * T, T)
        shift = jnp.broadcast_to(x_v[s, pl.ds(0, 16), cols].astype(F32)[:1], (16, T))
        for d in range(0, D, 16):
            xc = x_v[s, pl.ds(d, 16), cols].astype(F32) - shift
            s1, s2 = (s1 + xc, s2 + xc * xc) if d else (xc, xc * xc)
        m = jnp.sum(s1, axis=0, keepdims=True) * (1.0 / D)
        v = jnp.maximum(jnp.sum(s2, axis=0, keepdims=True) * (1.0 / D) - m * m, 0.0)
        m = jnp.broadcast_to(_round_bf16(m + shift[:1]), (16, T))
        inv = jnp.broadcast_to(
            1.0 / _round_bf16(jnp.sqrt(_round_bf16(_round_bf16(v) + 1e-5))), (16, T))
        for d in range(0, D, 16):
            x = x_v[s + zero, pl.ds(d, 16), cols].astype(F32)
            xn_v[s, pl.ds(d, 16), cols] = (_round_bf16(x - m) * inv).astype(BF16)
        return marker(xn_v[s + zero, :16, cols])

    def transpose_weight(i, lo=0, hi=D):
        for c in range(lo, hi, T):
            n = min(T, D - c)
            wt_v[pl.ds((i * D + c) // 2, n // 2), pl.ds(0, D)] = pltpu.bitcast(
                wraw_v[i, :, pl.ds(c, n)].T, U32)

    def transpose_wo(c):
        wt_v[pl.ds(WO, D // 2), pl.ds(c, T)] = pltpu.bitcast(wo_v[pl.ds(c, T), :].T, U32)

    def proj(s, row, n, keep=None):
        w = wt_v[pl.ds(row if not isinstance(row, int) else row // 2, n // 2), pl.ds(0, D)]
        mark = marks.pop(0) if len(marks) > 1 else None
        w = _bf(w if mark is None else tied(w, mark))
        return _dot(w.astype(F32)[:keep] if keep else w, xn_v[s])

    def project_q(s, p):
        zpad = jnp.zeros((GP - GR, L), F32)
        row32 = _iota((32, L), 0)
        slot = _iota((16, T), 1) >> 5
        q = proj(s, p * CH, CH)
        for j in range(2):
            g = 2 * p + j
            qg = q[j * GR:(j + 1) * GR]
            if s:
                pq_v[s, g] = _pack(jnp.concatenate([_phi(qg), zpad], axis=0))
            qg = jnp.concatenate([qg * QSCALE, zpad], axis=0)
            qh = [_pack(jnp.where((row32 >= 2 * h) & (row32 < 2 * h + DH), qg[16 * h:16 * h + 32], 0.0))
                  for h in range(HG)]
            for t in range(0, L, T):
                cols = pl.ds(t, T)
                rot = [pltpu.roll(w[:, t:t + T], h * QT, 1) if h else w[:, t:t + T]
                       for h, w in enumerate(qh)]
                for h in range(HG):
                    qs_v[s, g, h, :, cols] = rot[h]
                    qx_v[s, g, pl.ds(16 * (h // 2 + h % 2 * 2), 16), cols] = jnp.where(
                        ((slot - h) & 3) >= 2, rot[h], 0)
                for c in (1, 3):
                    ws = [jnp.where(slot == (c + h) % HG, rot[h], 0) for h in range(HG)]
                    qx_v[s, g, pl.ds(44 + 20 * c, 40), cols] = jnp.concatenate(
                        [ws[0][:8], *[a[8:] | b[:8] for a, b in zip(ws, ws[1:])], ws[-1][8:]], axis=0)
        marks.append(marker(qs_v[s + zero, g, 0, :8, :T], qx_v[s + zero, g, :8, :T],
                            *([pq_v[s + zero, g, :8, :T]] if s else [])))

    def project_k(s, p):
        k = proj(s, D + p * CH, CH)
        for j in range(2):
            kg = jnp.concatenate([k[j * GR:(j + 1) * GR], jnp.zeros((T - GR, L), F32)], axis=0)
            kn_v[s, 2 * p + j] = pltpu.bitcast(kg.astype(BF16).T, U32)
        marks.append(marker(kn_v[s + zero, 2 * p, :8, :]))

    def project_v(s, p):
        extra = 16 if p == NCH - 1 else 0
        row = 2 * D + p * CH
        if extra and s == NSEG - 1:
            row = pl.multiple_of(row // 2 + 8 * zero, 8)
        v = proj(s, row, CH + extra, CH + 8 if extra else None)
        for j in range(2):
            vt_v[s, 2 * p + j] = v[j * GR:(j + 1) * GR]
        if extra:
            r_v[s] = v[CH:CH + 8]
        marks.append(None)

    def mem_update(s, g):
        row, lane = _iota((GP, T), 0), _iota((GP, T), 1)
        keep = None
        for h in range(HG):
            rows = ((row >= h * DH) & (row < (h + 1) * DH)) | (row == GR + h)
            block = rows & (lane >= h * DH) & (lane < (h + 1) * DH)
            keep = keep | block if h else block
        pk = _phi(_bf(kn_v[s, g]).astype(F32))
        z = jnp.broadcast_to(jnp.sum(pk, axis=0, keepdims=True), (GP - GR, T))
        upd = jnp.where(keep, jnp.concatenate([_dot(vt_v[s, g], pk.astype(BF16)), z], axis=0), 0.0)
        mz_v[s, g] = mz_v[s - 1, g] + upd if s else upd

    def mem_read(s, g):
        mem_v[s - 1, g] = _dot(mz_v[s - 1, g, :, pl.ds(0, GP)], _bf(pq_v[s, g]))

    def project(f, s, ps=range(NCH), then=()):
        def step(p):
            f(s, p)
            for g in (2 * p, 2 * p + 1):
                for fn, seg in then:
                    fn(seg, g)

        return [partial(step, p) for p in ps]

    def run(dots, norm=None):
        for i, f in enumerate(dots):
            f()
            for t in range(i * NT // len(dots), (i + 1) * NT // len(dots)) if norm else ():
                mark = layernorm(norm, t)
                marks[-1] = mark if marks[-1] is None else marks[-1] | mark

    def small_tables():
        wt_v[pl.ds(3 * D // 2, 8), pl.ds(0, D)] = _pack(
            jnp.broadcast_to(wr_v[...].astype(F32).reshape(1, D), (16, D)))
        sg = jax.nn.sigmoid(beta_v[...].astype(F32).reshape(1, H))
        row = _iota((NG * 8, H), 0)
        head = (row >> 3) * HG + ((row + jnp.where((row & 4) != 0, 3, 0)) & 3)
        gate = jnp.sum(jnp.where(_iota((NG * 8, H), 1) == head,
                                 jnp.broadcast_to(sg, (NG * 8, H)), 0.0), axis=1, keepdims=True)
        gate = jnp.where((_iota((NG * 8, 1), 0) & 4) != 0, 1.0 - gate, gate)
        gate_v[...] = jnp.broadcast_to(gate, (NG * 8, T))

    def top2():
        r = _round_bf16(jnp.concatenate([r_v[s] for s in range(NSEG)], axis=1))
        pos = _iota((8, S), 1)
        m1 = jnp.max(r, axis=1, keepdims=True)
        i1 = jnp.min(jnp.where(r == m1, pos, S), axis=1, keepdims=True)
        r2 = jnp.where(pos == i1, -jnp.inf, r)
        m2 = jnp.max(r2, axis=1, keepdims=True)
        i2 = jnp.min(jnp.where((r2 == m2) & (pos != i1), pos, S), axis=1, keepdims=True)
        sub = _iota((8, S), 0)
        onehot = jnp.where(((sub == 0) & (pos == i1)) | ((sub == 1) & (pos == i2)), 1.0, 0.0)
        for s in range(NSEG):
            ot_v[s, pl.ds(D, 8), :] = onehot[:, s * L:(s + 1) * L]
        rs_v[...] = jnp.broadcast_to(
            jax.nn.sigmoid(jnp.where(_iota((8, 1), 0) == 0, m1, m2)), (8, T))
        return [jnp.clip(jnp.min(i), 0, S - 1) for i in (i1, i2)]

    def gather(tokens, d):
        n = min(L, D - d)
        for c, tok in enumerate(tokens):
            tile = xn_v[tok >> 9, pl.ds(d, n), pl.ds(pl.multiple_of(tok & (L - T), T), T)]
            pick = (_iota((8, T), 0) == c) & (_iota((8, T), 1) == (tok & (T - 1)))
            row = _dot_nt(jnp.where(pick, 1.0, 0.0), tile)
            rows = row + rows if c else row
        xs_v[:, pl.ds(d, n)] = rows
        y_v[:, pl.ds(d, n)] = jnp.zeros((8, n), F32)

    def ffn_steps(c):
        cols = pl.ds(c, L)
        acc = {}

        def gate_up(m, d):
            rows = pl.ds(d, min(T, D - d))
            a = _dot(xs_v[:, rows], (wg_v, wu_v)[m][rows, cols])
            acc[m] = a + acc[m] if d else a

        def down(d):
            rows = pl.ds(d, min(T, D - d))
            if d == 0:
                acc[2] = acc[0] * jax.nn.sigmoid(acc[0]) * acc[1]
            y_v[:, rows] += _dot_nt(acc[2], wd_v[rows, cols])

        return ([partial(gate_up, m, d) for m in range(2) for d in range(0, D, T)]
                + [partial(down, d) for d in range(0, D, T)])

    def ffn_wait():
        for c in ffn_cp:
            c.wait()

    def ffn_done():
        y = y_v[...] * rs_v[:, pl.ds(0, 1)]
        wo_v[pl.ds(D, DP - D), :] = jnp.concatenate(
            [y, jnp.zeros((DP - D - 8, D), F32)], axis=0).astype(BF16)
        transpose_wo(DP - T)

    tiles = [(s, i, j) for s in range(NSEG) for i in reversed(range(NT)) for j in range(i + 1)]

    def attend(groups, true_max, side=()):
        blocks = [(k, *t) for k in range(len(groups)) for t in tiles]
        row8 = _iota((8, T), 0)
        st, col_max, acc = {}, {}, {}

        def scores(n):
            k, s, i, j = blocks[n]
            cols = pl.ds(i * T, T)

            def qk(lo, cnt, q, first):
                parts = [jnp.zeros((first // 2, T), U32), q,
                         jnp.zeros(((T - first) // 2 - q.shape[0], T), U32)]
                return _dot(_bf(kn_v[s, groups[k], pl.ds((j * T + lo) // 2, cnt // 2), :]),
                            _bf(jnp.concatenate([p for p in parts if p.shape[0]], axis=0)))

            def bias(r):
                return bias_v[pl.ds(T + r * QT, QT), :]

            for h in range(HG):
                q = qs_v[s, groups[k], h, :, cols]
                if true_max:
                    t = qk(0, T, q, 16 * h)
                    if j == i:
                        t = t + pltpu.roll(bias_v[pl.ds(0, T), :], h * QT, 1)
                    st[n, h] = t
                    m = jnp.max(t, axis=0, keepdims=True)
                    col_max[s, i, h] = jnp.maximum(col_max[s, i, h], m) if j else m
                elif j + 1 < i:
                    st[n, h] = qk(0, T, q, 16 * h)
                elif j < i:
                    t = qk(0, T + QT, q, 16 * h)
                    st[n, h], st[n + 1, h] = t[:T], t[T:] + bias(h)
                elif i == 0:
                    st[n, h] = qk(0, QT, q, 16 * h) + bias(h)
            if j == i and not true_max:
                for h in range(2):
                    t = qk(QT, 2 * QT, qx_v[s, groups[k], pl.ds(32 * h, 32), cols], 16 * h)
                    st[n, 'pair', h] = t[:QT], t[QT:] + bias(4 + h)
                for c in (1, 3):
                    st[n, 'quad', c] = bias(6) + qk(
                        c * QT, QT, qx_v[s, groups[k], pl.ds(44 + 20 * c, 40), cols], 0)

        def probs(n):
            k, s, i, j = blocks[n]
            if true_max:
                return [jnp.exp2(st.pop((n, h)) - col_max[s, i, h]) for h in range(HG)]
            if j < i:
                return [jnp.exp2(st.pop((n, h))) for h in range(HG)]
            slot = _iota((QT, T), 1) >> 5
            quad = {c: jnp.exp2(st.pop((n, 'quad', c))) for c in (1, 3)}
            pair = [[jnp.exp2(t) for t in st.pop((n, 'pair', h))] for h in range(2)]
            out = []
            for h in range(HG):
                late = ((slot - h) & 3) >= 2
                out.append(jnp.concatenate([
                    jnp.exp2(st.pop((n, h))),
                    jnp.where(late, pair[h % 2][0], jnp.where(slot == (1 + h) % HG, quad[1], 0.0)),
                    jnp.where(late, pair[h % 2][1], 0.0),
                    jnp.where(slot == (3 + h) % HG, quad[3], 0.0)], axis=0))
            return out

        def values(n):
            k, s, i, j = blocks[n]
            for h, p in enumerate(probs(n)):
                w = vt_v[s, groups[k], pl.ds(16 * h, 24), pl.ds(j * T, T)]
                if h < HG - 1:
                    w = jnp.concatenate([w[:16], jnp.where(row8 == 5 + h, 1.0, w[16:])], axis=0)
                else:
                    w = jnp.concatenate([jnp.where(row8 == 4, 1.0, w[:8]), w[8:]], axis=0)
                a = _dot(w, p.astype(BF16))
                acc[h] = a + acc[h] if j else a
                if j == i:
                    acc_v[s, groups[k], pl.ds(24 * h, 24), pl.ds(i * T, T)] = acc[h]

        lag = NT + 1 if true_max else LAG
        for n in range(len(blocks)):
            step = n % (len(tiles) // NSEG)
            scores(n)
            if n >= lag:
                values(n - lag)
            if side and n >= FFN_FIRST_STEP and step in FFN_STEPS:
                side.pop(0)()
        assert not side
        return [partial(values, n) for n in range(len(blocks) - lag, len(blocks))]

    def finish(g, s, i, seg):
        row8 = _iota((8, T), 0)
        cols = pl.ds(i * T, T)
        acc = [acc_v[seg, g, pl.ds(24 * h, 24), cols] for h in range(HG)]
        acc = [pltpu.roll(t, T - h * QT, 1) if h else t for h, t in enumerate(acc)]
        sums = jnp.where(row8 < 5, acc[3][:8], acc[2][16:])
        den = sums = jnp.where(row8 == 5, acc[0][16:], jnp.where(row8 == 6, acc[1][16:], sums))
        if s > 0:
            mem = mem_v[s - 1, g, :, cols]
            den = jnp.where(row8 < 4, mem[GR:] + 1e-6, sums)
        coef = gate_v[pl.ds(_aligned(g * 8, 8), 8), :] / den

        def spread(lo, mid, hi):
            out = [lo[0], mid[0]]
            for h in range(1, HG):
                out += [jnp.where(row8 < 2 * h, hi[h - 1], lo[h]), mid[h]]
            return jnp.concatenate(out + [hi[HG - 1]], axis=0)

        cl = [jnp.broadcast_to(coef[r:r + 1], (8, T)) for r in (5, 6, 7, 4)]
        o = spread(*[[t[r:r + 8] for t in acc] for r in (0, 8, 16)]) * spread(cl, cl, cl)
        if s > 0:
            cm = [jnp.broadcast_to(coef[r:r + 1], (8, T)) for r in range(HG)]
            o = o + mem[:GR] * spread(cm, cm, cm)
        ot_v[s, pl.ds(_aligned(g * GR, 8), GR), cols] = o
        return sums

    def output(finish_segment, tail=()):
        pieces = [(s, 0, D) for s in range(NSEG - 1)]
        pieces += [(NSEG - 1, r, n) for r, n in ((0, 288), (288, 192), (480, 96))]
        out_cp = []
        finish_segment(0)
        for i, (s, r, n) in enumerate(pieces):
            rows = pl.ds(r, n)
            if s + 1 < NSEG:
                finish_segment(s + 1)
            att = _dot(_bf(wt_v[pl.ds(WO + r // 2, n // 2), :]), ot_v[s].astype(BF16))
            for f in tail if i == 0 else ():
                f()
            if s + 2 < NSEG:
                acc_v[0, 0, :8, :T] = att[-8:, :T]
            out_v[s, rows, :] = (x_v[s, rows, :].astype(F32) + att
                                 + xn_v[s, rows, :].astype(F32)).astype(BF16)
            out_cp.append(pltpu.make_async_copy(
                out_v.at[s, rows, :], out_hbm.at[rows, pl.ds(s * L, L)], out_sem.at[i]))
            out_cp[-1].start()
        return out_cp

    bias_v[pl.ds(0, T), :] = jnp.where(_iota((T, T), 0) <= _iota((T, T), 1), 0.0, NEG)
    for i, (rot, width) in enumerate([(h, T) for h in range(HG)] + [(0, 2 * QT), (1, 2 * QT), (0, QT)]):
        bias_v[pl.ds(T + i * QT, QT), :] = jnp.where(
            _iota((QT, T), 0) <= ((_iota((QT, T), 1) - rot * QT) & (width - 1)), 0.0, NEG)
    for s in range(NSEG):
        ot_v[s, pl.ds(D + 8, DP - D - 8), :] = jnp.zeros((DP - D - 8, L), F32)

    x_cp[0].wait()
    for t in range(NT):
        layernorm(0, t)
    wv_cp.wait()
    transpose_weight(2, 0, HEAD)
    project_v(0, 0)
    wv_rest_cp.wait()
    transpose_weight(2, HEAD)
    run(project(project_v, 0, range(1, 3)))
    for c in [*small_cp, wq_cp]:
        c.wait()
    small_tables()
    project_v(0, 3)
    transpose_weight(0)
    run(project(project_q, 0, range(3)))
    for c in [wk_cp, x_cp[1]]:
        c.wait()
    project_q(0, 3)
    transpose_weight(1)
    run(project(project_k, 0, range(3)), norm=1)
    run(project(project_k, 0, [3]) + project(project_k, 1, then=[(mem_update, 0)])
        + project(project_v, 1, [0]))
    for c in [*x_cp[2:], wo_cp]:
        c.wait()
    run(project(project_v, 1, range(1, 4)) + project(project_q, 1, range(3)), norm=2)
    project_q(1, 3)
    for c in range(0, DP - T, T):
        transpose_wo(c)
    run(project(project_v, 2) + project(project_k, 2), norm=3)
    run(project(project_q, 2) + project(project_v, 3, [3]))
    tokens = top2()
    run(project(project_k, 3, then=[(mem_update, 1)]) + project(project_q, 3, then=[(mem_read, 1)])
        + project(project_v, 3, [0, 1], then=[(mem_update, 2), (mem_read, 2)]))
    project_v(3, 2)
    for g in range(NG // 2, NG):
        mem_update(2, g)
        mem_read(2, g)
    for g in range(NG):
        mem_read(3, g)
    for d in range(0, D, L):
        gather(tokens, d)

    tail = attend(list(range(NG)), False,
                  [ffn_wait] + [f for c in range(0, FF, L) for f in ffn_steps(c)] + [ffn_done])

    lim = []

    def finish_and_watch(s):
        for g in range(NG):
            for i in range(NT):
                sums = finish(g, s, i, s + zero if s >= 2 else s)
                lim[:] = [jnp.minimum(lim[0], sums), jnp.maximum(lim[1], sums)] if lim else [sums, sums]

    out_cp = output(finish_and_watch, tail)
    safe = (_iota((8, T), 0) < 4) | ((lim[0] >= SAFE_LO) & (lim[1] <= SAFE_HI))
    unsafe = jnp.min(jnp.where(safe, 1, 0)) == 0
    for c in out_cp:
        c.wait()

    @pl.when(unsafe)
    def _():
        def redo(g, carry):
            for f in attend([g], True):
                f()
            for s in range(NSEG):
                for i in range(NT):
                    finish(g, s, i, s)
            return carry

        jax.lax.fori_loop(0, NG, redo, 0)
        for c in output(lambda s: None):
            c.wait()


@jax.jit
def pallas_parallel_sum__memory_aug_infini_attn__moe_arch_mod__prompt_kernel(
    A_x: jax.Array,
    A_wq: jax.Array,
    A_wk: jax.Array,
    A_wv: jax.Array,
    A_wo: jax.Array,
    A_beta: jax.Array,
    B_x: jax.Array,
    B_w_r: jax.Array,
    B_w_gate: jax.Array,
    B_w_up: jax.Array,
    B_w_down: jax.Array,
):
    del B_x
    assert A_x.shape == (1, S, D) and B_w_gate.shape == (D, FF)
    hbm = pl.BlockSpec(memory_space=pl.ANY)
    out_t = pl.pallas_call(
        _kernel,
        out_shape=jax.ShapeDtypeStruct((D, S), BF16),
        in_specs=[hbm] * 10,
        out_specs=hbm,
        scratch_shapes=[
            pltpu.VMEM((D,), BF16),
            pltpu.VMEM((H,), BF16),
            pltpu.VMEM((NSEG, D, L), BF16),
            pltpu.VMEM((3, D, D), BF16),
            pltpu.VMEM((DP, D), BF16),
            pltpu.VMEM((WO + D // 2, DP), U32),
            pltpu.VMEM((NSEG, D, L), BF16),
            pltpu.VMEM((NSEG, NG, HG, 16, L), U32),
            pltpu.VMEM((NSEG, NG, 144, L), U32),
            pltpu.VMEM((NSEG, NG, GP // 2, L), U32),
            pltpu.VMEM((NSEG, NG, L // 2, T), U32),
            pltpu.VMEM((NSEG, NG, GR, L), F32),
            pltpu.VMEM((NSEG, NG, HG * 24, L), F32),
            pltpu.VMEM((NSEG - 1, NG, GP, T), F32),
            pltpu.VMEM((NSEG - 1, NG, GP, L), F32),
            pltpu.VMEM((NSEG, DP, L), F32),
            pltpu.VMEM((NSEG, 8, L), F32),
            pltpu.VMEM((NG * 8, T), F32),
            pltpu.VMEM((T + 7 * QT, T), F32),
            pltpu.VMEM((8, D), F32),
            pltpu.VMEM((8, D), F32),
            pltpu.VMEM((8, T), F32),
            pltpu.VMEM((D, FF), BF16),
            pltpu.VMEM((D, FF), BF16),
            pltpu.VMEM((D, FF), BF16),
            pltpu.VMEM((NSEG, D, L), BF16),
            pltpu.SemaphoreType.DMA((NSEG + 10,)),
            pltpu.SemaphoreType.DMA((NSEG + 2,)),
        ],
        compiler_params=pltpu.CompilerParams(vmem_limit_bytes=100 * 2 ** 20),
        name="infini_mod",
    )(B_w_r, A_beta, A_x[0].T, A_wq, A_wk, A_wv, A_wo, B_w_gate, B_w_up, B_w_down.T)
    return out_t.T[None]
```

```python
import math
from functools import partial

import jax
import jax.numpy as jnp
import jax.experimental.pallas as pl
import jax.experimental.pallas.tpu as pltpu

D = 576
S = 2048
H = 32
DH = D // H
NSEG = 4
L = S // NSEG
FF = 4608
HG = 4
NG = H // HG
GR = HG * DH
GP = 80
T = 128
QT = T // HG
NT = L // T
CH = 2 * GR
NCH = D // CH
DP = 640
HEAD = 3 * T
WO = 3 * D // 2 + 8

F32 = jnp.float32
BF16 = jnp.bfloat16
U32 = jnp.uint32
QSCALE = (DH ** -0.5) * math.log2(math.e)
NEG = -1e30
SAFE_LO, SAFE_HI = 2.0 ** -30, 2.0 ** 30
LAG = 2
FFN_FIRST_STEP = 30
FFN_STEPS = (0, 1, 2, 4, 5, 7)


def _iota(shape, dim):
    return jax.lax.broadcasted_iota(jnp.int32, shape, dim)


def _round_bf16(t):
    return t.astype(BF16).astype(F32)


def _pack(t):
    return pltpu.bitcast(t.astype(BF16), U32)


def _bf(t):
    return pltpu.bitcast(t, BF16)


def _phi(t):
    return jnp.where(t > 0, t + 1.0, jnp.exp(t))


def _dot(a, b):
    return jax.lax.dot_general(a, b, (((1,), (0,)), ((), ())), preferred_element_type=F32)


def _dot_nt(a, b):
    return jax.lax.dot_general(a, b, (((1,), (1,)), ((), ())), preferred_element_type=F32)


def _aligned(i, n):
    return i if isinstance(i, int) else pl.multiple_of(i, n)


def _kernel(wr_hbm, beta_hbm, x_hbm, wq_hbm, wk_hbm, wv_hbm, wo_hbm, wg_hbm, wu_hbm, wd_hbm,
            out_hbm,
            wr_v, beta_v, x_v, wraw_v, wo_v, wt_v, xn_v, qs_v, qx_v, pq_v, kn_v, vt_v, acc_v,
            mz_v, mem_v, ot_v, r_v, gate_v, bias_v, xs_v, y_v, rs_v, wg_v, wu_v, wd_v, out_v,
            in_sem, out_sem):
    x_cp = [pltpu.make_async_copy(x_hbm.at[:, pl.ds(s * L, L)], x_v.at[s], in_sem.at[s])
            for s in range(NSEG)]
    head, rest = pl.ds(0, HEAD), pl.ds(HEAD, D - HEAD)
    wq_cp, wk_cp, wv_cp, wv_rest_cp, wo_cp, *more_cp = [
        pltpu.make_async_copy(src, dst, in_sem.at[NSEG + i]) for i, (src, dst) in enumerate((
            (wq_hbm, wraw_v.at[0]), (wk_hbm, wraw_v.at[1]),
            (wv_hbm.at[:, head], wraw_v.at[2, :, head]), (wv_hbm.at[:, rest], wraw_v.at[2, :, rest]),
            (wo_hbm, wo_v.at[pl.ds(0, D)]), (wr_hbm, wr_v), (beta_hbm, beta_v),
            (wg_hbm, wg_v), (wu_hbm, wu_v), (wd_hbm, wd_v)))]
    small_cp, ffn_cp = more_cp[:2], more_cp[2:]
    for c in [x_cp[0], wv_cp, wv_rest_cp, *small_cp, wq_cp, wk_cp, *x_cp[1:], wo_cp, *ffn_cp]:
        c.start()

    zero = jnp.min(_iota((8, T), 1))
    zeros = _iota((8, T), 1) * zero
    marks = []

    def marker(*values):
        out = pltpu.bitcast(values[0], jnp.int32)
        for t in values[1:]:
            out = out | pltpu.bitcast(t, jnp.int32)
        return out & zeros

    def tied(t, mark):
        head = pltpu.bitcast(pltpu.bitcast(t[:8, :T], jnp.int32) | mark, t.dtype)
        return jnp.concatenate([jnp.concatenate([head, t[:8, T:]], axis=1), t[8:]], axis=0)

    def layernorm(s, t):
        cols = pl.ds(t * T, T)
        shift = jnp.broadcast_to(x_v[s, pl.ds(0, 16), cols].astype(F32)[:1], (16, T))
        for d in range(0, D, 16):
            xc = x_v[s, pl.ds(d, 16), cols].astype(F32) - shift
            s1, s2 = (s1 + xc, s2 + xc * xc) if d else (xc, xc * xc)
        m = jnp.sum(s1, axis=0, keepdims=True) * (1.0 / D)
        v = jnp.maximum(jnp.sum(s2, axis=0, keepdims=True) * (1.0 / D) - m * m, 0.0)
        m = jnp.broadcast_to(_round_bf16(m + shift[:1]), (16, T))
        inv = jnp.broadcast_to(
            1.0 / _round_bf16(jnp.sqrt(_round_bf16(_round_bf16(v) + 1e-5))), (16, T))
        for d in range(0, D, 16):
            x = x_v[s + zero, pl.ds(d, 16), cols].astype(F32)
            xn_v[s, pl.ds(d, 16), cols] = (_round_bf16(x - m) * inv).astype(BF16)
        return marker(xn_v[s + zero, :16, cols])

    def transpose_weight(i, lo=0, hi=D):
        for c in range(lo, hi, T):
            n = min(T, D - c)
            wt_v[pl.ds((i * D + c) // 2, n // 2), pl.ds(0, D)] = pltpu.bitcast(
                wraw_v[i, :, pl.ds(c, n)].T, U32)

    def transpose_wo(c):
        wt_v[pl.ds(WO, D // 2), pl.ds(c, T)] = pltpu.bitcast(wo_v[pl.ds(c, T), :].T, U32)

    def proj(s, row, n, keep=None):
        w = wt_v[pl.ds(row if not isinstance(row, int) else row // 2, n // 2), pl.ds(0, D)]
        mark = marks.pop(0) if len(marks) > 1 else None
        w = _bf(w if mark is None else tied(w, mark))
        return _dot(w.astype(F32)[:keep] if keep else w, xn_v[s])

    def project_q(s, p):
        zpad = jnp.zeros((GP - GR, L), F32)
        row32 = _iota((32, L), 0)
        slot = _iota((16, T), 1) >> 5
        q = proj(s, p * CH, CH)
        for j in range(2):
            g = 2 * p + j
            qg = q[j * GR:(j + 1) * GR]
            if s:
                pq_v[s, g] = _pack(jnp.concatenate([_phi(qg), zpad], axis=0))
            qg = jnp.concatenate([qg * QSCALE, zpad], axis=0)
            qh = [_pack(jnp.where((row32 >= 2 * h) & (row32 < 2 * h + DH), qg[16 * h:16 * h + 32], 0.0))
                  for h in range(HG)]
            for t in range(0, L, T):
                cols = pl.ds(t, T)
                rot = [pltpu.roll(w[:, t:t + T], h * QT, 1) if h else w[:, t:t + T]
                       for h, w in enumerate(qh)]
                for h in range(HG):
                    qs_v[s, g, h, :, cols] = rot[h]
                    qx_v[s, g, pl.ds(16 * (h // 2 + h % 2 * 2), 16), cols] = jnp.where(
                        ((slot - h) & 3) >= 2, rot[h], 0)
                for c in (1, 3):
                    ws = [jnp.where(slot == (c + h) % HG, rot[h], 0) for h in range(HG)]
                    qx_v[s, g, pl.ds(44 + 20 * c, 40), cols] = jnp.concatenate(
                        [ws[0][:8], *[a[8:] | b[:8] for a, b in zip(ws, ws[1:])], ws[-1][8:]], axis=0)
        marks.append(marker(qs_v[s + zero, g, 0, :8, :T], qx_v[s + zero, g, :8, :T],
                            *([pq_v[s + zero, g, :8, :T]] if s else [])))

    def project_k(s, p):
        k = proj(s, D + p * CH, CH)
        for j in range(2):
            kg = jnp.concatenate([k[j * GR:(j + 1) * GR], jnp.zeros((T - GR, L), F32)], axis=0)
            kn_v[s, 2 * p + j] = pltpu.bitcast(kg.astype(BF16).T, U32)
        marks.append(marker(kn_v[s + zero, 2 * p, :8, :]))

    def project_v(s, p):
        extra = 16 if p == NCH - 1 else 0
        row = 2 * D + p * CH
        if extra and s == NSEG - 1:
            row = pl.multiple_of(row // 2 + 8 * zero, 8)
        v = proj(s, row, CH + extra, CH + 8 if extra else None)
        for j in range(2):
            vt_v[s, 2 * p + j] = v[j * GR:(j + 1) * GR]
        if extra:
            r_v[s] = v[CH:CH + 8]
        marks.append(None)

    def mem_update(s, g):
        row, lane = _iota((GP, T), 0), _iota((GP, T), 1)
        keep = None
        for h in range(HG):
            rows = ((row >= h * DH) & (row < (h + 1) * DH)) | (row == GR + h)
            block = rows & (lane >= h * DH) & (lane < (h + 1) * DH)
            keep = keep | block if h else block
        pk = _phi(_bf(kn_v[s, g]).astype(F32))
        z = jnp.broadcast_to(jnp.sum(pk, axis=0, keepdims=True), (GP - GR, T))
        upd = jnp.where(keep, jnp.concatenate([_dot(vt_v[s, g], pk.astype(BF16)), z], axis=0), 0.0)
        mz_v[s, g] = mz_v[s - 1, g] + upd if s else upd

    def mem_read(s, g):
        mem_v[s - 1, g] = _dot(mz_v[s - 1, g, :, pl.ds(0, GP)], _bf(pq_v[s, g]))

    def project(f, s, ps=range(NCH), then=()):
        def step(p):
            f(s, p)
            for g in (2 * p, 2 * p + 1):
                for fn, seg in then:
                    fn(seg, g)

        return [partial(step, p) for p in ps]

    def run(dots, norm=None):
        for i, f in enumerate(dots):
            f()
            for t in range(i * NT // len(dots), (i + 1) * NT // len(dots)) if norm else ():
                mark = layernorm(norm, t)
                marks[-1] = mark if marks[-1] is None else marks[-1] | mark

    def small_tables():
        wt_v[pl.ds(3 * D // 2, 8), pl.ds(0, D)] = _pack(
            jnp.broadcast_to(wr_v[...].astype(F32).reshape(1, D), (16, D)))
        sg = jax.nn.sigmoid(beta_v[...].astype(F32).reshape(1, H))
        row = _iota((NG * 8, H), 0)
        head = (row >> 3) * HG + ((row + jnp.where((row & 4) != 0, 3, 0)) & 3)
        gate = jnp.sum(jnp.where(_iota((NG * 8, H), 1) == head,
                                 jnp.broadcast_to(sg, (NG * 8, H)), 0.0), axis=1, keepdims=True)
        gate = jnp.where((_iota((NG * 8, 1), 0) & 4) != 0, 1.0 - gate, gate)
        gate_v[...] = jnp.broadcast_to(gate, (NG * 8, T))

    def top2():
        r = _round_bf16(jnp.concatenate([r_v[s] for s in range(NSEG)], axis=1))
        pos = _iota((8, S), 1)
        m1 = jnp.max(r, axis=1, keepdims=True)
        i1 = jnp.min(jnp.where(r == m1, pos, S), axis=1, keepdims=True)
        r2 = jnp.where(pos == i1, -jnp.inf, r)
        m2 = jnp.max(r2, axis=1, keepdims=True)
        i2 = jnp.min(jnp.where((r2 == m2) & (pos != i1), pos, S), axis=1, keepdims=True)
        sub = _iota((8, S), 0)
        onehot = jnp.where(((sub == 0) & (pos == i1)) | ((sub == 1) & (pos == i2)), 1.0, 0.0)
        for s in range(NSEG):
            ot_v[s, pl.ds(D, 8), :] = onehot[:, s * L:(s + 1) * L]
        rs_v[...] = jnp.broadcast_to(
            jax.nn.sigmoid(jnp.where(_iota((8, 1), 0) == 0, m1, m2)), (8, T))
        return [jnp.clip(jnp.min(i), 0, S - 1) for i in (i1, i2)]

    def gather(tokens, d):
        n = min(L, D - d)
        for c, tok in enumerate(tokens):
            tile = xn_v[tok >> 9, pl.ds(d, n), pl.ds(pl.multiple_of(tok & (L - T), T), T)]
            pick = (_iota((8, T), 0) == c) & (_iota((8, T), 1) == (tok & (T - 1)))
            row = _dot_nt(jnp.where(pick, 1.0, 0.0), tile)
            rows = row + rows if c else row
        xs_v[:, pl.ds(d, n)] = rows
        y_v[:, pl.ds(d, n)] = jnp.zeros((8, n), F32)

    def ffn_steps(c):
        cols = pl.ds(c, L)
        acc = {}

        def gate_up(m, d):
            rows = pl.ds(d, min(T, D - d))
            a = _dot(xs_v[:, rows], (wg_v, wu_v)[m][rows, cols])
            acc[m] = a + acc[m] if d else a

        def down(d):
            rows = pl.ds(d, min(T, D - d))
            if d == 0:
                acc[2] = acc[0] * jax.nn.sigmoid(acc[0]) * acc[1]
            y_v[:, rows] += _dot_nt(acc[2], wd_v[rows, cols])

        return ([partial(gate_up, m, d) for m in range(2) for d in range(0, D, T)]
                + [partial(down, d) for d in range(0, D, T)])

    def ffn_wait():
        for c in ffn_cp:
            c.wait()

    def ffn_done():
        y = y_v[...] * rs_v[:, pl.ds(0, 1)]
        wo_v[pl.ds(D, DP - D), :] = jnp.concatenate(
            [y, jnp.zeros((DP - D - 8, D), F32)], axis=0).astype(BF16)
        transpose_wo(DP - T)

    tiles = [(s, i, j) for s in range(NSEG) for i in reversed(range(NT)) for j in range(i + 1)]

    def attend(groups, true_max, side=()):
        blocks = [(k, *t) for k in range(len(groups)) for t in tiles]
        row8 = _iota((8, T), 0)
        st, col_max, acc = {}, {}, {}

        def scores(n):
            k, s, i, j = blocks[n]
            cols = pl.ds(i * T, T)

            def qk(lo, cnt, q, first):
                parts = [jnp.zeros((first // 2, T), U32), q,
                         jnp.zeros(((T - first) // 2 - q.shape[0], T), U32)]
                return _dot(_bf(kn_v[s, groups[k], pl.ds((j * T + lo) // 2, cnt // 2), :]),
                            _bf(jnp.concatenate([p for p in parts if p.shape[0]], axis=0)))

            def bias(r):
                return bias_v[pl.ds(T + r * QT, QT), :]

            for h in range(HG):
                q = qs_v[s, groups[k], h, :, cols]
                if true_max:
                    t = qk(0, T, q, 16 * h)
                    if j == i:
                        t = t + pltpu.roll(bias_v[pl.ds(0, T), :], h * QT, 1)
                    st[n, h] = t
                    m = jnp.max(t, axis=0, keepdims=True)
                    col_max[s, i, h] = jnp.maximum(col_max[s, i, h], m) if j else m
                elif j + 1 < i:
                    st[n, h] = qk(0, T, q, 16 * h)
                elif j < i:
                    t = qk(0, T + QT, q, 16 * h)
                    st[n, h], st[n + 1, h] = t[:T], t[T:] + bias(h)
                elif i == 0:
                    st[n, h] = qk(0, QT, q, 16 * h) + bias(h)
            if j == i and not true_max:
                for h in range(2):
                    t = qk(QT, 2 * QT, qx_v[s, groups[k], pl.ds(32 * h, 32), cols], 16 * h)
                    st[n, 'pair', h] = t[:QT], t[QT:] + bias(4 + h)
                for c in (1, 3):
                    st[n, 'quad', c] = bias(6) + qk(
                        c * QT, QT, qx_v[s, groups[k], pl.ds(44 + 20 * c, 40), cols], 0)

        def probs(n):
            k, s, i, j = blocks[n]
            if true_max:
                return [jnp.exp2(st.pop((n, h)) - col_max[s, i, h]) for h in range(HG)]
            if j < i:
                return [jnp.exp2(st.pop((n, h))) for h in range(HG)]
            slot = _iota((QT, T), 1) >> 5
            quad = {c: jnp.exp2(st.pop((n, 'quad', c))) for c in (1, 3)}
            pair = [[jnp.exp2(t) for t in st.pop((n, 'pair', h))] for h in range(2)]
            out = []
            for h in range(HG):
                late = ((slot - h) & 3) >= 2
                out.append(jnp.concatenate([
                    jnp.exp2(st.pop((n, h))),
                    jnp.where(late, pair[h % 2][0], jnp.where(slot == (1 + h) % HG, quad[1], 0.0)),
                    jnp.where(late, pair[h % 2][1], 0.0),
                    jnp.where(slot == (3 + h) % HG, quad[3], 0.0)], axis=0))
            return out

        def values(n):
            k, s, i, j = blocks[n]
            for h, p in enumerate(probs(n)):
                w = vt_v[s, groups[k], pl.ds(16 * h, 24), pl.ds(j * T, T)]
                if h < HG - 1:
                    w = jnp.concatenate([w[:16], jnp.where(row8 == 5 + h, 1.0, w[16:])], axis=0)
                else:
                    w = jnp.concatenate([jnp.where(row8 == 4, 1.0, w[:8]), w[8:]], axis=0)
                a = _dot(w, p.astype(BF16))
                acc[h] = a + acc[h] if j else a
                if j == i:
                    acc_v[s, groups[k], pl.ds(24 * h, 24), pl.ds(i * T, T)] = acc[h]

        lag = NT + 1 if true_max else LAG
        for n in range(len(blocks)):
            step = n % (len(tiles) // NSEG)
            scores(n)
            if n >= lag:
                values(n - lag)
            if side and n >= FFN_FIRST_STEP and step in FFN_STEPS:
                side.pop(0)()
        assert not side
        return [partial(values, n) for n in range(len(blocks) - lag, len(blocks))]

    def finish(g, s, i, seg):
        row8 = _iota((8, T), 0)
        cols = pl.ds(i * T, T)
        acc = [acc_v[seg, g, pl.ds(24 * h, 24), cols] for h in range(HG)]
        acc = [pltpu.roll(t, T - h * QT, 1) if h else t for h, t in enumerate(acc)]
        sums = jnp.where(row8 < 5, acc[3][:8], acc[2][16:])
        den = sums = jnp.where(row8 == 5, acc[0][16:], jnp.where(row8 == 6, acc[1][16:], sums))
        if s > 0:
            mem = mem_v[s - 1, g, :, cols]
            den = jnp.where(row8 < 4, mem[GR:] + 1e-6, sums)
        coef = gate_v[pl.ds(_aligned(g * 8, 8), 8), :] / den

        def spread(lo, mid, hi):
            out = [lo[0], mid[0]]
            for h in range(1, HG):
                out += [jnp.where(row8 < 2 * h, hi[h - 1], lo[h]), mid[h]]
            return jnp.concatenate(out + [hi[HG - 1]], axis=0)

        cl = [jnp.broadcast_to(coef[r:r + 1], (8, T)) for r in (5, 6, 7, 4)]
        o = spread(*[[t[r:r + 8] for t in acc] for r in (0, 8, 16)]) * spread(cl, cl, cl)
        if s > 0:
            cm = [jnp.broadcast_to(coef[r:r + 1], (8, T)) for r in range(HG)]
            o = o + mem[:GR] * spread(cm, cm, cm)
        ot_v[s, pl.ds(_aligned(g * GR, 8), GR), cols] = o
        return sums

    def output(finish_segment, tail=()):
        pieces = [(s, 0, D) for s in range(NSEG - 1)]
        pieces += [(NSEG - 1, r, n) for r, n in ((0, 288), (288, 192), (480, 96))]
        out_cp, probe = [], 0.0
        finish_segment(0)
        for i, (s, r, n) in enumerate(pieces):
            rows = pl.ds(r, n)
            if s + 1 < NSEG:
                finish_segment(s + 1)
            att = _dot(_bf(wt_v[pl.ds(WO + r // 2, n // 2), :]), ot_v[s].astype(BF16))
            if r == 0:
                probe = jnp.abs(att[:8]) + probe
            for f in tail if i == 0 else ():
                f()
            if s + 2 < NSEG:
                acc_v[0, 0, :8, :T] = att[-8:, :T]
            out_v[s, rows, :] = (x_v[s, rows, :].astype(F32) + att
                                 + xn_v[s, rows, :].astype(F32)).astype(BF16)
            out_cp.append(pltpu.make_async_copy(
                out_v.at[s, rows, :], out_hbm.at[rows, pl.ds(s * L, L)], out_sem.at[i]))
            out_cp[-1].start()
        return out_cp, probe

    bias_v[pl.ds(0, T), :] = jnp.where(_iota((T, T), 0) <= _iota((T, T), 1), 0.0, NEG)
    for i, (rot, width) in enumerate([(h, T) for h in range(HG)] + [(0, 2 * QT), (1, 2 * QT), (0, QT)]):
        bias_v[pl.ds(T + i * QT, QT), :] = jnp.where(
            _iota((QT, T), 0) <= ((_iota((QT, T), 1) - rot * QT) & (width - 1)), 0.0, NEG)
    for s in range(NSEG):
        ot_v[s, pl.ds(D + 8, DP - D - 8), :] = jnp.zeros((DP - D - 8, L), F32)

    x_cp[0].wait()
    for t in range(NT):
        layernorm(0, t)
    wv_cp.wait()
    transpose_weight(2, 0, HEAD)
    project_v(0, 0)
    wv_rest_cp.wait()
    transpose_weight(2, HEAD)
    run(project(project_v, 0, range(1, 3)))
    for c in [*small_cp, wq_cp]:
        c.wait()
    small_tables()
    project_v(0, 3)
    transpose_weight(0)
    run(project(project_q, 0, range(3)))
    for c in [wk_cp, x_cp[1]]:
        c.wait()
    project_q(0, 3)
    transpose_weight(1)
    run(project(project_k, 0, range(3)), norm=1)
    run(project(project_k, 0, [3]) + project(project_k, 1, then=[(mem_update, 0)])
        + project(project_v, 1, [0]))
    for c in [*x_cp[2:], wo_cp]:
        c.wait()
    run(project(project_v, 1, range(1, 4)) + project(project_q, 1, range(3)), norm=2)
    project_q(1, 3)
    for c in range(0, DP - T, T):
        transpose_wo(c)
    run(project(project_v, 2) + project(project_k, 2), norm=3)
    run(project(project_q, 2) + project(project_v, 3, [3]))
    tokens = top2()
    run(project(project_k, 3, then=[(mem_update, 1)]) + project(project_q, 3, then=[(mem_read, 1)])
        + project(project_v, 3, [0, 1], then=[(mem_update, 2), (mem_read, 2)]))
    project_v(3, 2)
    for g in range(NG // 2, NG):
        mem_update(2, g)
        mem_read(2, g)
    for g in range(NG):
        mem_read(3, g)
    for d in range(0, D, L):
        gather(tokens, d)

    tail = attend(list(range(NG)), False,
                  [ffn_wait] + [f for c in range(0, FF, L) for f in ffn_steps(c)] + [ffn_done])

    lim = []

    def finish_and_watch(s):
        for g in range(NG):
            for i in range(NT):
                sums = finish(g, s, i, s + zero if s >= 2 else s)
                lim[:] = [jnp.minimum(lim[0], sums), jnp.maximum(lim[1], sums)] if lim else [sums, sums]

    out_cp, probe = output(finish_and_watch, tail)
    safe = (_iota((8, T), 0) < 4) | ((lim[0] >= SAFE_LO) & (lim[1] <= SAFE_HI))
    for t in range(0, L, T):
        safe = safe & (probe[:, t:t + T] < jnp.inf)
    unsafe = jnp.min(jnp.where(safe, 1, 0)) == 0
    for c in out_cp:
        c.wait()

    @pl.when(unsafe)
    def _():
        def redo(g, carry):
            for f in attend([g], True):
                f()
            for s in range(NSEG):
                for i in range(NT):
                    finish(g, s, i, s)
            return carry

        jax.lax.fori_loop(0, NG, redo, 0)
        for c in output(lambda s: None)[0]:
            c.wait()


@jax.jit
def pallas_parallel_sum__memory_aug_infini_attn__moe_arch_mod__prompt_kernel(
    A_x: jax.Array,
    A_wq: jax.Array,
    A_wk: jax.Array,
    A_wv: jax.Array,
    A_wo: jax.Array,
    A_beta: jax.Array,
    B_x: jax.Array,
    B_w_r: jax.Array,
    B_w_gate: jax.Array,
    B_w_up: jax.Array,
    B_w_down: jax.Array,
):
    del B_x
    assert A_x.shape == (1, S, D) and B_w_gate.shape == (D, FF)
    hbm = pl.BlockSpec(memory_space=pl.ANY)
    out_t = pl.pallas_call(
        _kernel,
        out_shape=jax.ShapeDtypeStruct((D, S), BF16),
        in_specs=[hbm] * 10,
        out_specs=hbm,
        scratch_shapes=[
            pltpu.VMEM((D,), BF16),
            pltpu.VMEM((H,), BF16),
            pltpu.VMEM((NSEG, D, L), BF16),
            pltpu.VMEM((3, D, D), BF16),
            pltpu.VMEM((DP, D), BF16),
            pltpu.VMEM((WO + D // 2, DP), U32),
            pltpu.VMEM((NSEG, D, L), BF16),
            pltpu.VMEM((NSEG, NG, HG, 16, L), U32),
            pltpu.VMEM((NSEG, NG, 144, L), U32),
            pltpu.VMEM((NSEG, NG, GP // 2, L), U32),
            pltpu.VMEM((NSEG, NG, L // 2, T), U32),
            pltpu.VMEM((NSEG, NG, GR, L), F32),
            pltpu.VMEM((NSEG, NG, HG * 24, L), F32),
            pltpu.VMEM((NSEG - 1, NG, GP, T), F32),
            pltpu.VMEM((NSEG - 1, NG, GP, L), F32),
            pltpu.VMEM((NSEG, DP, L), F32),
            pltpu.VMEM((NSEG, 8, L), F32),
            pltpu.VMEM((NG * 8, T), F32),
            pltpu.VMEM((T + 7 * QT, T), F32),
            pltpu.VMEM((8, D), F32),
            pltpu.VMEM((8, D), F32),
            pltpu.VMEM((8, T), F32),
            pltpu.VMEM((D, FF), BF16),
            pltpu.VMEM((D, FF), BF16),
            pltpu.VMEM((D, FF), BF16),
            pltpu.VMEM((NSEG, D, L), BF16),
            pltpu.SemaphoreType.DMA((NSEG + 10,)),
            pltpu.SemaphoreType.DMA((NSEG + 2,)),
        ],
        compiler_params=pltpu.CompilerParams(vmem_limit_bytes=100 * 2 ** 20),
        name="infini_mod",
    )(B_w_r, A_beta, A_x[0].T, A_wq, A_wk, A_wv, A_wo, B_w_gate, B_w_up, B_w_down.T)
    return out_t.T[None]
```
